```python
import jax
import jax.numpy as jnp

def _softmax(x, axis=-1):
    return jax.nn.softmax(x, axis=axis)
def _gelu(x):
    return jax.nn.gelu(x, approximate=True)
def _silu(x):
    return jax.nn.silu(x)
def _sigmoid(x):
    return jax.nn.sigmoid(x)
def _layernorm(x, axis=-1, eps=1e-5):
    m = jnp.mean(x, axis=axis, keepdims=True)
    v = jnp.var(x, axis=axis, keepdims=True)
    return (x - m) / jnp.sqrt(v + eps)
def _scatter_add(tgt, idx, src, axis=0):
    return tgt.at[idx].add(src)
def _segment_sum(src, seg, n):
    return jax.ops.segment_sum(src, seg, n)
class _Rng:
    def __init__(self, key):
        self._k = key
    def _next(self):
        self._k, sub = jax.random.split(self._k)
        return sub
    def normal(self, shape):
        return jax.random.normal(self._next(), shape, dtype=jnp.bfloat16)
    def randint(self, lo, hi, shape):
        return jax.random.randint(self._next(), shape, lo, hi, dtype=jnp.int32)
    def uniform(self, shape, lo=0.0, hi=1.0):
        return jax.random.uniform(self._next(), shape, jnp.bfloat16, lo, hi)
    def permutation(self, n):
        return jax.random.permutation(self._next(), n)


kernel_name = 'gated_mix__linear_attn_block__moe_arch_mod__prompt'

def setup_inputs():
    _rng = _Rng(jax.random.key(int.from_bytes(__import__("os").urandom(4), "little")))
    _w = (lambda a: (lambda t: t.astype(jnp.bfloat16) if jnp.issubdtype(t.dtype, jnp.floating) else t)(jnp.asarray(a)))
    def _A_setup():
        B, S, D = 1, 2048, 1024
        return {
            "x": _w((lambda *s: _rng.normal(s) * 0.05)(B, S, D)),
            "wqkv": _w((lambda *s: _rng.normal(s) * 0.05)(D, 3 * D)),
            "wo": _w((lambda *s: _rng.normal(s) * 0.05)(D, D)),
        }
    _A_in = _A_setup()

    def _B_setup():
        B, S, D, F, C = 1, 2048, 1024, 3584, 1
        return {
            "x": _w((lambda *s: _rng.normal(s) * 0.05)(B, S, D)),
            "w_r": _w((lambda *s: _rng.normal(s) * 0.05)(D)),
            "w_gate": _w((lambda *s: _rng.normal(s) * 0.05)(D, F)),
            "w_up": _w((lambda *s: _rng.normal(s) * 0.05)(D, F)),
            "w_down": _w((lambda *s: _rng.normal(s) * 0.05)(F, D)),
        }
    _B_in = _B_setup()

    return {
        "A_x": _A_in["x"],
        "A_wqkv": _A_in["wqkv"],
        "A_wo": _A_in["wo"],
        "B_x": _B_in["x"],
        "B_w_r": _B_in["w_r"],
        "B_w_gate": _B_in["w_gate"],
        "B_w_up": _B_in["w_up"],
        "B_w_down": _B_in["w_down"],
        "gate_w": _w((lambda *s: _rng.normal(s) * 0.05)(1024)),
    }

def reference(A_x, A_wqkv, A_wo, B_x, B_w_r, B_w_gate, B_w_up, B_w_down, gate_w):
    def _A_ref(x, wqkv, wo):
        B, S, D = x.shape
        H = 32; Dh = D // H
        qkv = (lambda x, *d: x.transpose(*d))((x @ wqkv).reshape(B, S, 3, H, Dh), 2, 0, 3, 1, 4)
        q, k, v = qkv[0], qkv[1], qkv[2]
        phi = lambda t: jnp.where(t > 0, t + 1, jnp.exp(t)) + 1e-6
        pq, pk = phi(q), phi(k)
        kv = jnp.einsum("bhsd,bhse->bhde", pk, v)
        z = jnp.einsum("bhsd->bhd", pk)
        num = jnp.einsum("bhqd,bhde->bhqe", pq, kv)
        den = jnp.einsum("bhqd,bhd->bhq", pq, z)[..., None] + 1e-6
        o = num / den
        return (lambda x, *d: x.transpose(*d))(o, 0, 2, 1, 3).reshape(B, S, D) @ wo

    def _B_ref(x, w_r, w_gate, w_up, w_down):
        B, S, D = x.shape
        C = 1
        r = x @ w_r
        idx = jnp.argsort(-r, axis=-1)[:, :C]
        idx_e = jnp.repeat(idx.reshape(B, C, 1), D, axis=2)
        x_sel = jnp.take_along_axis(x, idx_e, axis=1)
        g = _silu(x_sel @ w_gate)
        u = x_sel @ w_up
        y = (g * u) @ w_down
        r_sel = _sigmoid(jnp.take_along_axis(r, idx, axis=1))
        y = y * r_sel.reshape(B, C, 1)
        b_off = (jnp.arange(B) * S).reshape(B, 1)
        flat_idx = (idx + b_off).reshape(B * C)
        zero = (x * 0.0).reshape(B * S, D)
        upd = _scatter_add(zero, flat_idx, y.reshape(B * C, D), axis=0)
        return x + upd.reshape(B, S, D)

    x = A_x
    g = _sigmoid((x * gate_w).sum(-1, keepdims=True))
    a = _A_ref(x, A_wqkv, A_wo)
    b = _B_ref(x, B_w_r, B_w_gate, B_w_up, B_w_down)
    return g * a + (1 - g) * b
```

```python
import jax
import jax.numpy as jnp
from jax import lax
import jax.experimental.pallas as pl
import jax.experimental.pallas.tpu as pltpu

S, D, F, H, DH = 2048, 1024, 3584, 32, 32
TS = 512
NT = S // TS
MC = 256
PC = 256
NP = D // PC
FC = F // NP
OC = 256
DO_FFN = True
f32, bf16 = jnp.float32, jnp.bfloat16
NT_DIMS = (((1,), (1,)), ((), ()))


def _phi(t):
    return jnp.where(t > 0, t + 1.0, jnp.exp(t)) + 1e-6


def _sigmoid(t):
    return 1.0 / (1.0 + jnp.exp(-t))


def _kernel(ax_hbm, wqkv_hbm, wo_hbm, bx_hbm, wr_ref, wg_hbm, wu_hbm, wd_hbm, gw_ref, out_hbm,
            x_v, w_v, wo_v, bx_v, wg_v, wu_v, wd_v, wT_v, pkT_v, pq_v, z_v, m_v, xcol_v, y_v, o_v,
            sem_x, sem_w, sem_b, sem_f, sem_o):
    def x_cp(t):
        return pltpu.make_async_copy(ax_hbm.at[0, pl.ds(t * TS, TS)], x_v.at[t], sem_x.at[t])

    def w_cp(j):
        return pltpu.make_async_copy(wqkv_hbm.at[:, pl.ds(j * D, D)], w_v.at[j], sem_w.at[j])

    wo_cp = pltpu.make_async_copy(wo_hbm, wo_v, sem_w.at[3])
    bx_cp = pltpu.make_async_copy(bx_hbm.at[0], bx_v, sem_b.at[0])

    def f_cp(j):
        return (pltpu.make_async_copy(wg_hbm.at[:, pl.ds(j * FC, FC)], wg_v.at[j], sem_f.at[0, j]),
                pltpu.make_async_copy(wu_hbm.at[:, pl.ds(j * FC, FC)], wu_v.at[j], sem_f.at[1, j]),
                pltpu.make_async_copy(wd_hbm.at[pl.ds(j * FC, FC)], wd_v.at[j], sem_f.at[2, j]))

    def o_cp(t):
        return pltpu.make_async_copy(o_v.at[t], out_hbm.at[0, pl.ds(t * TS, TS)], sem_o.at[t])

    w_cp(1).start()
    x_cp(0).start()
    for t in range(1, NT):
        x_cp(t).start()
    w_cp(0).start()
    bx_cp.start()

    def transpose_w(j):
        for c in range(D // 256):
            wT_v[j, pl.ds(c * 256, 256), :] = w_v[j, :, pl.ds(c * 256, 256)].T

    w_cp(1).wait()
    transpose_w(1)
    z_v[...] = jnp.zeros_like(z_v)

    def k_body(t, c):
        x_cp(t).wait()
        xt = x_v[t]
        for m in range(D // MC):
            rows = pl.ds(m * MC, MC)
            kT = lax.dot_general(wT_v[1, rows, :], xt, NT_DIMS, preferred_element_type=f32)
            pk = _phi(kT)
            zs = pk[:, 0:128]
            for l in range(1, TS // 128):
                zs = zs + pk[:, l * 128:(l + 1) * 128]
            z_v[rows, :] += zs
            pkT_v[t, rows, :] = pk.astype(bf16)
        return c
    lax.fori_loop(0, NT, k_body, 0)

    w_cp(2).start()
    wo_cp.start()
    for j in range(NP):
        for cp in f_cp(j):
            cp.start()

    z_v[...] = jnp.broadcast_to(jnp.sum(z_v[...], axis=1, keepdims=True), z_v.shape)
    w_cp(0).wait()
    transpose_w(0)
    bx_cp.wait()

    wr = wr_ref[...].astype(f32)

    def q_body(t, carry):
        best, bidx = carry
        xt = x_v[t]
        for m in range(D // MC):
            rows = pl.ds(m * MC, MC)
            qT = lax.dot_general(wT_v[0, rows, :], xt, NT_DIMS, preferred_element_type=f32)
            pq = _phi(qT)
            zc = z_v[rows, :]
            zc = jnp.concatenate([zc] * (TS // 128), axis=1)
            den = jnp.sum((pq * zc).reshape(MC // DH, DH, TS), axis=1, keepdims=True) + 1e-6
            pqn = (pq.reshape(MC // DH, DH, TS) * (1.0 / den)).reshape(MC, TS)
            pq_v[t, :, rows] = pqn.astype(bf16).T
        r = jnp.sum(bx_v[pl.ds(pl.multiple_of(t * TS, TS), TS), :].astype(f32) * wr, axis=1, keepdims=True)
        r = r.astype(bf16).astype(f32)
        mx = jnp.max(r)
        ids = lax.broadcasted_iota(jnp.int32, (TS, 1), 0) + t * TS
        mi = jnp.min(jnp.where(r == mx, ids, S))
        upd = mx > best
        return jnp.where(upd, mx, best), jnp.where(upd, mi, bidx)
    best, bidx = lax.fori_loop(0, NT, q_body, (jnp.float32(-jnp.inf), jnp.int32(0)))

    base = pl.multiple_of((bidx // 16) * 16, 16)
    slab = bx_v[pl.ds(base, 16), :].astype(f32)
    sel = lax.broadcasted_iota(jnp.int32, (16, D), 0) == (bidx - base)
    xsel = jnp.sum(jnp.where(sel, slab, 0.0), axis=0, keepdims=True)
    xcol_v[...] = jnp.broadcast_to(xsel, (128, D)).T
    y_v[...] = jnp.zeros_like(y_v)

    w_cp(2).wait()
    wo_cp.wait()

    def p_body(j, c):
        rows = pl.ds(pl.multiple_of(j * PC, PC), PC)
        p = jnp.dot(pkT_v[0, rows, :], x_v[0], preferred_element_type=f32)
        for t in range(1, NT):
            p += jnp.dot(pkT_v[t, rows, :], x_v[t], preferred_element_type=f32)
        m_v[rows, :] = p.astype(bf16)
        if DO_FFN:
            for cp in f_cp(j):
                cp.wait()
            ga = jnp.zeros((8, FC), f32)
            ua = jnp.zeros((8, FC), f32)
            for r in range(D // 16):
                xc = xcol_v[pl.ds(r * 16, 16), :]
                xc = jnp.concatenate([xc] * (FC // 128), axis=1)
                pg = wg_v[j, pl.ds(r * 16, 16), :].astype(f32) * xc
                pu = wu_v[j, pl.ds(r * 16, 16), :].astype(f32) * xc
                ga += pg[0:8] + pg[8:16]
                ua += pu[0:8] + pu[8:16]
            g = jnp.sum(ga, axis=0, keepdims=True)
            u = jnp.sum(ua, axis=0, keepdims=True)
            h = g * _sigmoid(g) * u
            hcol = jnp.broadcast_to(h, (128, FC)).T
            ya = y_v[...]
            for r in range(FC // 16):
                hc = jnp.concatenate([hcol[r * 16:(r + 1) * 16]] * (D // 128), axis=1)
                pd = wd_v[j, pl.ds(r * 16, 16), :].astype(f32) * hc
                ya += pd[0:8] + pd[8:16]
            y_v[...] = ya
        return c
    lax.fori_loop(0, NP, p_body, 0)
    if not DO_FFN:
        for j in range(NP):
            for cp in f_cp(j):
                cp.wait()

    blk = (lax.broadcasted_iota(jnp.int32, (128, 128), 0) // DH) == (lax.broadcasted_iota(jnp.int32, (128, 128), 1) // DH)
    for g in range(D // 128):
        rows = pl.ds(g * 128, 128)
        kv = jnp.dot(m_v[rows, :], w_v[2, :, rows], preferred_element_type=f32)
        kv = jnp.where(blk, kv, 0.0).astype(bf16)
        m_v[rows, :] = jnp.dot(kv, wo_v[rows, :], preferred_element_type=f32).astype(bf16)

    y = jnp.sum(y_v[...], axis=0, keepdims=True) * _sigmoid(jnp.full((1, D), best, f32))
    bx_v[pl.ds(base, 16), :] = jnp.where(sel, slab + y, slab).astype(bf16)

    gw = gw_ref[...].astype(f32)

    def o_body(t, c):
        for m in range(TS // OC):
            rows = pl.ds(m * OC, OC)
            a = jnp.dot(pq_v[t, rows, :], m_v[...], preferred_element_type=f32)
            g = _sigmoid(jnp.sum(x_v[t, rows, :].astype(f32) * gw, axis=1, keepdims=True))
            b = bx_v[pl.ds(pl.multiple_of(t * TS + m * OC, OC), OC), :].astype(f32)
            o_v[t, rows, :] = (g * a + (1.0 - g) * b).astype(bf16)
        o_cp(t).start()
        return c
    lax.fori_loop(0, NT, o_body, 0)
    for t in range(NT):
        o_cp(t).wait()


@jax.jit
def pallas_gated_mix__linear_attn_block__moe_arch_mod__prompt_kernel(
        A_x, A_wqkv, A_wo, B_x, B_w_r, B_w_gate, B_w_up, B_w_down, gate_w):
    hbm = pl.BlockSpec(memory_space=pl.ANY)
    vmem = pl.BlockSpec(memory_space=pltpu.VMEM)
    return pl.pallas_call(
        _kernel,
        out_shape=jax.ShapeDtypeStruct((1, S, D), bf16),
        in_specs=[hbm, hbm, hbm, hbm, vmem, hbm, hbm, hbm, vmem],
        out_specs=hbm,
        scratch_shapes=[
            pltpu.VMEM((NT, TS, D), bf16),
            pltpu.VMEM((3, D, D), bf16),
            pltpu.VMEM((D, D), bf16),
            pltpu.VMEM((S, D), bf16),
            pltpu.VMEM((NP, D, FC), bf16),
            pltpu.VMEM((NP, D, FC), bf16),
            pltpu.VMEM((NP, FC, D), bf16),
            pltpu.VMEM((2, D, D), bf16),
            pltpu.VMEM((NT, D, TS), bf16),
            pltpu.VMEM((NT, TS, D), bf16),
            pltpu.VMEM((D, 128), f32),
            pltpu.VMEM((D, D), bf16),
            pltpu.VMEM((D, 128), f32),
            pltpu.VMEM((8, D), f32),
            pltpu.VMEM((NT, TS, D), bf16),
            pltpu.SemaphoreType.DMA((NT,)),
            pltpu.SemaphoreType.DMA((4,)),
            pltpu.SemaphoreType.DMA((1,)),
            pltpu.SemaphoreType.DMA((3, NP)),
            pltpu.SemaphoreType.DMA((NT,)),
        ],
        compiler_params=pltpu.CompilerParams(vmem_limit_bytes=100 * 1024 * 1024),
    )(A_x, A_wqkv, A_wo, B_x, B_w_r.reshape(1, D), B_w_gate, B_w_up, B_w_down, gate_w.reshape(1, D))
```

```python
import jax
import jax.numpy as jnp
from jax import lax
import jax.experimental.pallas as pl
import jax.experimental.pallas.tpu as pltpu

S, D, F, DH = 2048, 1024, 3584, 32
TS = 512
TH = TS // 2
NT = S // TS
HD = D // 2
MC = 128
NM = HD // MC
NP = HD // 128
FC = F // NP
TIE = True
FR = 128
OC = 128
f32, bf16, u32 = jnp.float32, jnp.bfloat16, jnp.uint32


def _phi(t):
    return jnp.where(t > 0, t + 1.0, jnp.exp(t)) + 1e-6


def _sigmoid(t):
    return 1.0 / (1.0 + jnp.exp(-t))


def _dot(a, b):
    return jnp.dot(a, b, preferred_element_type=f32)


def _dot_nt(a, b):
    return lax.dot_general(a, b, (((1,), (1,)), ((), ())), preferred_element_type=f32)


def _pack(v):
    return pltpu.bitcast(v.astype(bf16), u32)


def _pack2(even, odd):
    return pltpu.pack_elementwise([even, odd], packed_dtype=bf16)


def _pack_mixed(v):
    r, c = v.shape
    v = v.reshape(r // 16, 2, 8, c)
    return _pack2(v[:, 0].reshape(r // 2, c), v[:, 1].reshape(r // 2, c))


def _unpack(w):
    return pltpu.bitcast(w, bf16)


def _half(start, size):
    if isinstance(start, int):
        return pl.ds(start // 2, size // 2)
    return pl.ds(pl.multiple_of(start // 2, size // 2), size // 2)


def _left(a11, a12, a21, a22):
    return (a11 + a22, a21 + a22, a11, a22, a11 + a12, a21 - a11, a12 - a22)


def _right(b11, b12, b21, b22):
    return (b11 + b22, b11, b12 - b22, b21 - b11, b22, b11 + b12, b21 + b22)


def _strassen(prod, fill=()):
    fill = list(fill)
    n = len(fill)

    def p(i):
        m = prod(i)
        for w in fill[(n * i) // 7:(n * (i + 1)) // 7]:
            w()
        return m

    c11 = c22 = p(0)
    c21 = p(1)
    c22 = c22 - c21
    c12 = p(2)
    c22 = c22 + c12
    m = p(3)
    c11, c21 = c11 + m, c21 + m
    m = p(4)
    c11, c12 = c11 - m, c12 + m
    c22 = c22 + p(5)
    c11 = c11 + p(6)
    return c11, c12, c21, c22


def _kernel(x_hbm, wqkv_hbm, wo_hbm, bx_hbm, wr_ref, wg_hbm, wu_hbm, wd_hbm, gw_ref, out_hbm,
            x_v, wqk_v, wv_v, wo_v, bx_v, wg_v, wu_v, wd_v,
            xa_v, xb_v, wqs_v, wks_v, ks_v, qs_v, ms_v, z_v, zq_v, xcol_v, hcol_v, y_v, o_v,
            sem_x, sem_w, sem_v, sem_b, sem_f, sem_o):
    def x_cp(t):
        return pltpu.make_async_copy(x_hbm.at[0, pl.ds(t * TS, TS)], x_v.at[t], sem_x.at[t])

    def w_cp(j, m, h):
        return pltpu.make_async_copy(wqkv_hbm.at[:, pl.ds(j * D + h * HD + m * MC, MC)],
                                     wqk_v.at[j, m, h], sem_w.at[(j * NM + m) * 2 + h])

    def v_cp(g):
        return pltpu.make_async_copy(wqkv_hbm.at[:, pl.ds(2 * D + g * 128, 128)], wv_v.at[g], sem_v.at[g])

    wo_cp = pltpu.make_async_copy(wo_hbm, wo_v, sem_v.at[2 * NP])

    def b_cp(t):
        rows = pl.ds(t * TS, TS)
        return pltpu.make_async_copy(bx_hbm.at[0, rows], bx_v.at[rows], sem_b.at[t])

    def f_cp(j, i):
        cols = pl.ds(j * FC, FC)
        src = wd_hbm.at[cols] if i == 2 else (wg_hbm, wu_hbm)[i].at[:, cols]
        return pltpu.make_async_copy(src, (wg_v, wu_v, wd_v)[i].at[j], sem_f.at[i * NP + j])

    def o_cp(t, c):
        return pltpu.make_async_copy(o_v.at[t, pl.ds(c * OC, OC)], out_hbm.at[0, pl.ds(t * TS + c * OC, OC)],
                                     sem_o.at[t * (TS // OC) + c])

    def prep_w(j, m, k):
        blk = [wqk_v[j, m, h, pl.ds(i * HD + k * 128, 128), :].astype(f32).T for h in (0, 1) for i in (0, 1)]
        for i, a in enumerate(_left(*blk)):
            (wqs_v, wks_v)[j][i, _half(m * MC, MC), pl.ds(k * 128, 128)] = (_pack_mixed, _pack)[j](a)

    def prep_x(src, dst_v, dst, r, n):
        blk = [pltpu.bitcast(x_v[src, pl.ds(h * TH + r, n), pl.ds(i * HD, HD)], u32) for i in (0, 1) for h in (0, 1)]
        even, odd = (_right(*[pltpu.unpack_elementwise(b, index=p, packed_dtype=bf16, unpacked_dtype=f32)
                              for b in blk]) for p in (0, 1))
        for i in range(7):
            dst_v[dst, i, _half(r, n), :] = blk[0] if i == 1 else blk[3] if i == 4 else _pack2(even[i], odd[i])

    def project(w_v, xs_v, u, m, fill):
        rows = _half(m * MC, MC)
        c = _strassen(lambda i: _dot_nt(_unpack(w_v[i, rows, :]), _unpack(xs_v[u, i])), fill)
        return [_phi(b) for b in c]

    x_cp(0).start()
    for m in range(NM):
        for h in (0, 1):
            w_cp(1, m, h).start()
    x_cp(0).wait()
    x_cp(1).start()
    for r in range(0, TH, 64):
        prep_x(0, xa_v, 0, r, 64)
    z_v[...] = jnp.zeros_like(z_v)
    y_v[...] = jnp.zeros_like(y_v)
    for m in range(NM):
        for h in (0, 1):
            w_cp(1, m, h).wait()
        for h in (0, 1):
            w_cp(0, m, h).start()
        for k in range(HD // 128):
            prep_w(1, m, k)
    x_cp(2).start()

    def k_tile(t, u, cur_v, nxt_v, nxt):
        for h in (0, 1):
            w_cp(0, t, h).wait()
            v_cp(h * NP + t).start()
        b_cp(t).start()
        src = jnp.minimum(t + 1, NT - 1)
        for m in range(NM):
            n = TH // NM // 2
            fill = [lambda: prep_x(src, nxt_v, nxt, (2 * m) * n, n), lambda: prep_w(0, t, m),
                    lambda: prep_x(src, nxt_v, nxt, (2 * m + 1) * n, n)]
            c11, c12, c21, c22 = project(wks_v, cur_v, u, m, fill)
            for h, zs in enumerate((c11 + c12, c21 + c22)):
                zr = pl.ds(h * HD + m * MC, MC)
                z_v[zr, :] += sum(zs[:, l:l + 128] for l in range(128, TH, 128)) + zs[:, 0:128]
            for i, b in enumerate(_right(c11, c21, c12, c22)):
                ks_v[t, i, _half(m * MC, MC), :] = _pack_mixed(b)

    def k_body(u, carry):
        x_cp(2 * u + 1).wait()

        @pl.when(u == 0)
        def _():
            x_cp(3).start()

        k_tile(2 * u, u, xa_v, xb_v, u)

        @pl.when(u == 0)
        def _():
            x_cp(2).wait()

        k_tile(2 * u + 1, u, xb_v, xa_v, u + 1)
        return carry

    lax.fori_loop(0, NT // 2, k_body, 0)
    wo_cp.start()
    for r in range(0, D, 8):
        zq_v[pl.ds(r // 16 * 16 + r // 8 % 2, 8, stride=2), :] = jnp.broadcast_to(
            jnp.sum(z_v[pl.ds(r, 8), :], axis=1, keepdims=True), (8, 128))

    wr = wr_ref[...].astype(f32).reshape(1, D)
    row8 = lax.broadcasted_iota(jnp.int32, (8, 1), 0)

    def q_tile(t, u, xs_v, top):
        for i in range(3):
            f_cp(t, i).start()
        b_cp(t).wait()

        def score(r0, n):
            base = pl.multiple_of(t * TS + r0, n)
            r = jnp.sum(bx_v[pl.ds(base, n), :].astype(f32) * wr, axis=1, keepdims=True)
            r = r.astype(bf16).astype(f32)
            for i in range(0, n, 8):
                upd = r[i:i + 8] > top[0]
                top[0] = jnp.where(upd, r[i:i + 8], top[0])
                top[1] = jnp.where(upd, row8 + (base + i), top[1])

        for m in range(NM):
            n = TS // NM // 2
            c = project(wqs_v, xs_v, u, m, [lambda: score(2 * m * n, n), lambda: score((2 * m + 1) * n, n)])
            p = []
            for i, pq in enumerate(c):
                zc = zq_v[pl.ds((i // 2) * HD + m * MC, MC), :]
                zc = jnp.concatenate([zc] * (TH // 128), axis=1)
                den = jnp.sum((pq * zc).reshape(MC // DH, DH, TH), axis=1, keepdims=True) + 1e-6
                p.append((pq.reshape(MC // DH, DH, TH) * (1.0 / den)).reshape(MC, TH).T)
            for i, a in enumerate(_left(p[0], p[2], p[1], p[3])):
                qs_v[t, i, :, pl.ds(m * MC, MC)] = _pack(a)

    def q_body(u, carry):
        top = list(carry)
        q_tile(2 * u, u, xa_v, top)
        q_tile(2 * u + 1, u, xb_v, top)
        return tuple(top)

    best, bidx = lax.fori_loop(0, NT // 2, q_body, (jnp.full((8, 1), -jnp.inf, f32), row8))
    top_r = jnp.max(best)
    idx = jnp.min(jnp.where(best == top_r, bidx, S - 1))
    slab = pl.ds(pl.multiple_of((idx // 16) * 16, 16), 16)
    picked = lax.broadcasted_iota(jnp.int32, (16, D), 0) == idx % 16
    xsel = jnp.sum(jnp.where(picked, bx_v[slab, :].astype(f32), 0.0), axis=0, keepdims=True)
    xcol_v[...] = jnp.broadcast_to(xsel, (128, D)).T
    hcol_v[...] = jnp.zeros_like(hcol_v)
    for g in range(2 * NP):
        v_cp(g).wait()
    wo_cp.wait()
    f_cp(0, 2).wait()

    def matvec(acc, w_ref, j, col_ref, r0, n):
        for r in range(r0, r0 + n, 16):
            w = w_ref[j, pl.ds(r, 16), :].astype(f32)
            pr = w * jnp.concatenate([col_ref[pl.ds(r, 16), :]] * (w.shape[1] // 128), axis=1)
            acc[0] = acc[0] + (pr[0:8] + pr[8:16])
        return acc[0]

    zero = jnp.full((8, 128), idx >> 16, jnp.int32).astype(u32)

    def after(words, v):
        if not TIE:
            return words
        bits = pltpu.bitcast(v, u32)
        dep = zero
        for l in range(0, v.shape[1], 128):
            dep = dep & bits[:, l:l + 128]
        top = words[0:8] | jnp.concatenate([dep] * (words.shape[1] // 128), axis=1)
        return jnp.concatenate([top, words[8:]], axis=0)

    blk = (lax.broadcasted_iota(jnp.int32, (128, 128), 0) // DH) == (lax.broadcasted_iota(jnp.int32, (128, 128), 1) // DH)
    x_of = (0, 6, 1, 4, 5, 3, 2)

    def p_body(j, carry):
        f_cp(j, 0).wait()
        f_cp(j, 1).wait()
        prev = jnp.maximum(j - 1, 0)

        @pl.when(j > 1)
        def _():
            f_cp(prev, 2).wait()

        ga, ua, ya = [jnp.zeros((8, FC), f32)], [jnp.zeros((8, FC), f32)], [y_v[...]]
        fill = []
        for s in range(0, D, FR):
            fill.append(lambda s=s: matvec(ga, wg_v, j, xcol_v, s, FR))
            fill.append(lambda s=s: matvec(ua, wu_v, j, xcol_v, s, FR))
        for s in range(0, FC, FR):
            fill.append(lambda s=s: matvec(ya, wd_v, prev, hcol_v, s, FR))
        rows = _half(j * 128, 128)

        def prod(i):
            acc = None
            for t in range(NT):
                k = i * NT + t
                lhs = ks_v[t, i, rows, :]
                for w in fill[(k * len(fill)) // 28:((k + 1) * len(fill)) // 28]:
                    lhs = after(lhs, w())
                d = _dot(_unpack(lhs), _unpack((xa_v, xb_v)[t % 2][t // 2, x_of[i]]))
                acc = d if acc is None else acc + d
            return acc

        d11, d12, d21, d22 = _strassen(prod)
        y_v[...] = ya[0]
        g = jnp.sum(ga[0], axis=0, keepdims=True)
        u = jnp.sum(ua[0], axis=0, keepdims=True)
        hcol_v[...] = jnp.broadcast_to(g * _sigmoid(g) * u, (128, FC)).T
        ms = []
        for h, (lo, hi) in enumerate(((d11, d21), (d12, d22))):
            grp = h * NP + j
            kv = _dot(jnp.concatenate([lo, hi], axis=1).astype(bf16), wv_v[grp])
            kv = jnp.where(blk, kv, 0.0).astype(bf16)
            mh = _dot(kv, wo_v[pl.ds(pl.multiple_of(grp * 128, 128), 128), :])
            ms += [mh[:, :HD], mh[:, HD:]]
        for i, b in enumerate(_right(*ms)):
            ms_v[i, rows, :] = _pack(b)
        return carry

    lax.fori_loop(0, NP, p_body, 0)
    f_cp(NP - 1, 2).wait()
    ya = [y_v[...]]
    matvec(ya, wd_v, NP - 1, hcol_v, 0, FC)
    y = jnp.sum(ya[0], axis=0, keepdims=True) * _sigmoid(jnp.full((1, D), top_r, f32))
    old = bx_v[slab, :].astype(f32)
    bx_v[slab, :] = jnp.where(picked, old + y, old).astype(bf16)

    gw = gw_ref[...].astype(f32).reshape(1, D)

    def o_body(t, carry):
        for c in range(TH // OC):
            a = _strassen(lambda i: _dot(_unpack(qs_v[t, i, _half(c * OC, OC), :]), _unpack(ms_v[i])))
            for h in (0, 1):
                rows = pl.ds(h * TH + c * OC, OC)
                g = _sigmoid(jnp.sum(x_v[t, rows, :].astype(f32) * gw, axis=1, keepdims=True))
                b = bx_v[pl.ds(pl.multiple_of(t * TS + h * TH + c * OC, OC), OC), :].astype(f32)
                ah = jnp.concatenate([a[2 * h], a[2 * h + 1]], axis=1)
                o_v[t, rows, :] = (g * ah + (1.0 - g) * b).astype(bf16)
                o_cp(t, h * (TH // OC) + c).start()
        return carry

    lax.fori_loop(0, NT, o_body, 0)
    for t in range(NT):
        for c in range(TS // OC):
            o_cp(t, c).wait()


@jax.jit
def pallas_gated_mix__linear_attn_block__moe_arch_mod__prompt_kernel(
        A_x, A_wqkv, A_wo, B_x, B_w_r, B_w_gate, B_w_up, B_w_down, gate_w):
    hbm = pl.BlockSpec(memory_space=pl.ANY)
    vmem = pl.BlockSpec(memory_space=pltpu.VMEM)
    return pl.pallas_call(
        _kernel,
        out_shape=jax.ShapeDtypeStruct((1, S, D), bf16),
        in_specs=[hbm, hbm, hbm, hbm, vmem, hbm, hbm, hbm, vmem],
        out_specs=hbm,
        scratch_shapes=[
            pltpu.VMEM((NT, TS, D), bf16),
            pltpu.VMEM((2, NM, 2, D, MC), bf16),
            pltpu.VMEM((2 * NP, D, 128), bf16),
            pltpu.VMEM((D, D), bf16),
            pltpu.VMEM((S, D), bf16),
            pltpu.VMEM((NP, D, FC), bf16),
            pltpu.VMEM((NP, D, FC), bf16),
            pltpu.VMEM((NP, FC, D), bf16),
            pltpu.VMEM((NT // 2 + 1, 7, TH // 2, HD), u32),
            pltpu.VMEM((NT // 2, 7, TH // 2, HD), u32),
            pltpu.VMEM((7, HD // 2, HD), u32),
            pltpu.VMEM((7, HD // 2, HD), u32),
            pltpu.VMEM((NT, 7, HD // 2, TH), u32),
            pltpu.VMEM((NT, 7, TH // 2, HD), u32),
            pltpu.VMEM((7, HD // 2, HD), u32),
            pltpu.VMEM((D, 128), f32),
            pltpu.VMEM((D, 128), f32),
            pltpu.VMEM((D, 128), f32),
            pltpu.VMEM((FC, 128), f32),
            pltpu.VMEM((8, D), f32),
            pltpu.VMEM((NT, TS, D), bf16),
            pltpu.SemaphoreType.DMA((NT,)),
            pltpu.SemaphoreType.DMA((4 * NM,)),
            pltpu.SemaphoreType.DMA((2 * NP + 1,)),
            pltpu.SemaphoreType.DMA((NT,)),
            pltpu.SemaphoreType.DMA((3 * NP,)),
            pltpu.SemaphoreType.DMA((S // OC,)),
        ],
        compiler_params=pltpu.CompilerParams(vmem_limit_bytes=110 * 1024 * 1024),
    )(A_x, A_wqkv, A_wo, B_x, B_w_r, B_w_gate, B_w_up, B_w_down, gate_w)
```

```python
import jax
import jax.numpy as jnp
from jax import lax
import jax.experimental.pallas as pl
import jax.experimental.pallas.tpu as pltpu

S, D, F, DH = 2048, 1024, 3584, 32
TS = 512
TH = TS // 2
NT = S // TS
HD = D // 2
MC = 128
NM = HD // MC
NP = HD // 128
FC = F // NP
FO = 1200
FP = (NT - 1) * FO
DR = 48
PK = 28
CP = 5
FLAGS = None
FN = 7
FR = 128
OC = 64
f32, bf16, u32 = jnp.float32, jnp.bfloat16, jnp.uint32


def _phi(t):
    return jnp.maximum(t + 1e-6, 1e-6) + jnp.exp(jnp.minimum(t, 0.0))


def _sigmoid(t):
    return 1.0 / (1.0 + jnp.exp(-t))


def _dot(a, b):
    return jnp.dot(a, b, preferred_element_type=f32)


def _dot_nt(a, b):
    return lax.dot_general(a, b, (((1,), (1,)), ((), ())), preferred_element_type=f32)


def _pack(v):
    return pltpu.bitcast(v.astype(bf16), u32)


def _pack2(even, odd):
    return pltpu.pack_elementwise([even, odd], packed_dtype=bf16)


def _pack_mixed(v):
    r, c = v.shape
    v = v.reshape(r // 16, 2, 8, c)
    return _pack2(v[:, 0].reshape(r // 2, c), v[:, 1].reshape(r // 2, c))


def _unpack(w):
    return pltpu.bitcast(w, bf16)


def _half(start, size):
    if isinstance(start, int):
        return pl.ds(start // 2, size // 2)
    return pl.ds(pl.multiple_of(start // 2, size // 2), size // 2)


def _left(a11, a12, a21, a22):
    return (a11 + a22, a21 + a22, a11, a22, a11 + a12, a21 - a11, a12 - a22)


def _right(b11, b12, b21, b22):
    return (b11 + b22, b11, b12 - b22, b21 - b11, b22, b11 + b12, b21 + b22)


def _strassen(prod, fill=(), copies=None):
    fill = list(fill)
    n = len(fill)

    def p(i):
        m = prod(i)
        last = CP if copies else FN
        for w in fill[n * min(i, last) // last:n * min(i + 1, last) // last]:
            w(m)
        if copies and i == CP:
            copies(m)
        return m

    c11 = c22 = p(0)
    c21 = p(1)
    c22 = c22 - c21
    c12 = p(2)
    c22 = c22 + c12
    m = p(3)
    c11, c21 = c11 + m, c21 + m
    m = p(4)
    c11, c12 = c11 - m, c12 + m
    c22 = c22 + p(5)
    c11 = c11 + p(6)
    return c11, c12, c21, c22


def _kernel(x_hbm, wqkv_hbm, wo_hbm, bx_hbm, wr_ref, wg_hbm, wu_hbm, wd_hbm, gw_ref, out_hbm,
            x_v, wqk_v, wv_v, wo_v, bx_v, wg_v, wu_v, wd_v,
            xa_v, xb_v, wqs_v, wks_v, ks_v, qs_v, p_v, ms_v, z_v, zq_v, xcol_v, hcol_v, y_v, o_v,
            sem_x, sem_w, sem_v, sem_b, sem_f, sem_o):
    def x_cp(t):
        return pltpu.make_async_copy(x_hbm.at[0, pl.ds(t * TS, TS)], x_v.at[t], sem_x.at[t])

    def w_cp(j, m, h):
        return pltpu.make_async_copy(wqkv_hbm.at[:, pl.ds(j * D + h * HD + m * 128, 128)],
                                     wqk_v.at[j, m, h], sem_w.at[(j * NP + m) * 2 + h])

    def v_cp(g):
        return pltpu.make_async_copy(wqkv_hbm.at[:, pl.ds(2 * D + g * 128, 128)], wv_v.at[g], sem_v.at[g])

    wo_cp = pltpu.make_async_copy(wo_hbm, wo_v, sem_v.at[2 * NP])

    def b_cp(t):
        rows = pl.ds(t * TS, TS)
        return pltpu.make_async_copy(bx_hbm.at[0, rows], bx_v.at[rows], sem_b.at[t])

    def f_cp(j, i):
        cols = pl.ds(j * FC, FC)
        if i == 2:
            return pltpu.make_async_copy(wd_hbm.at[cols], wd_v.at[cols], sem_f.at[i * NP + j])
        return pltpu.make_async_copy((wg_hbm, wu_hbm)[i].at[:, cols], (wg_v, wu_v)[i].at[j], sem_f.at[i * NP + j])

    def o_cp(t, c):
        return pltpu.make_async_copy(o_v.at[t, pl.ds(c * OC, OC)], out_hbm.at[0, pl.ds(t * TS + c * OC, OC)],
                                     sem_o.at[t * (TS // OC) + c])

    def after(words, v):
        if v is None:
            return words
        dep = zero[0] & pltpu.bitcast(v[0:8, 0:128], u32)
        r, c = words.shape
        return (words.reshape(r // 8, 8, c) | jnp.concatenate([dep] * (c // 128), axis=1)).reshape(r, c)

    def words_of(block, v):
        return after(pltpu.bitcast(block, u32), v)

    def prep_w(j, m, k, v):
        blk = [_unpack(words_of(wqk_v[j, m, h, pl.ds(i * HD + k * 128, 128), :], v)).astype(f32).T
               for h in (0, 1) for i in (0, 1)]
        for i, a in enumerate(_left(*blk)):
            (wqs_v, wks_v)[j][i, _half(m * 128, 128), pl.ds(k * 128, 128)] = (_pack_mixed, _pack)[j](a)

    def prep_x(src, dst_v, dst, r, n, v):
        blk = [words_of(x_v[src, pl.ds(h * TH + r, n), pl.ds(i * HD, HD)], v) for i in (0, 1) for h in (0, 1)]
        even, odd = (_right(*[pltpu.unpack_elementwise(b, index=p, packed_dtype=bf16, unpacked_dtype=f32)
                              for b in blk]) for p in (0, 1))
        for i in range(7):
            dst_v[dst, i, _half(r, n), :] = blk[0] if i == 1 else blk[3] if i == 4 else _pack2(even[i], odd[i])

    def project(w_v, xs_v, u, m, fill, copies=None):
        rows = _half(m * MC, MC)
        return _strassen(lambda i: _dot_nt(_unpack(w_v[i, rows, :]), _unpack(xs_v[u, i])), fill, copies)

    def w_all(j, ms):
        return [w_cp(j, m, h) for m in ms for h in (0, 1)]

    def prep_ws(j, ms):
        return [lambda v, m=m, k=k: prep_w(j, m, k, v) for m in ms for k in range(HD // 128)]

    def prep_xs(t, r0, r1):
        return [lambda v, r=r: prep_x(t, (xa_v, xb_v)[t % 2], t // 2, r, 16, v) for r in range(r0, r1, 16)]

    def k_finish(t, m, c):
        c11, c12, c21, c22 = [_phi(b) for b in c]
        for h, zs in enumerate((c11 + c12, c21 + c22)):
            zr = pl.ds(h * HD + m * MC, MC)
            zs = sum(zs[:, l:l + 128] for l in range(128, TH, 128)) + zs[:, 0:128]
            z_v[zr, :] = zs if t == 0 else z_v[zr, :] + zs
        for i, b in enumerate(_right(c11, c21, c12, c22)):
            ks_v[t, i, _half(m * MC, MC), :] = _pack_mixed(b)

    def sync(waits, starts):
        def run(_):
            for cp in waits:
                cp.wait()
            for cp in starts:
                cp.start()
        return run

    plan = {
        (0, 0): (prep_ws(1, [1]), sync(w_all(1, [2, 3]), [x_cp(2)])),
        (0, 1): (prep_ws(1, [2, 3]), sync([x_cp(1)], w_all(0, [0, 1]))),
        (0, 2): (prep_xs(1, 0, TH // 2), None),
        (0, 3): (prep_xs(1, TH // 2, TH), sync([x_cp(2)], [x_cp(3)] + w_all(0, [2, 3]) + [b_cp(0), b_cp(1)])),
        (1, 0): (prep_xs(2, 0, TH // 4), None),
        (1, 1): (prep_xs(2, TH // 4, TH // 2), None),
        (1, 2): (prep_xs(2, TH // 2, 3 * TH // 4), None),
        (1, 3): (prep_xs(2, 3 * TH // 4, TH),
                 sync([x_cp(3)] + w_all(0, range(NP)),
                      [b_cp(2), b_cp(3)] + [v_cp(g) for g in range(2 * NP)] + [wo_cp, f_cp(0, 0), f_cp(0, 1)])),
        (2, 0): (prep_xs(3, 0, TH // 4), None),
        (2, 1): (prep_xs(3, TH // 4, TH // 2), None),
        (2, 2): (prep_xs(3, TH // 2, 3 * TH // 4), None),
        (2, 3): (prep_xs(3, 3 * TH // 4, TH), None),
        (3, 0): (prep_ws(0, [0]), None),
        (3, 1): (prep_ws(0, [1]), None),
        (3, 2): (prep_ws(0, [2]), None),
        (3, 3): (prep_ws(0, [3]), None),
    }
    for cp in [x_cp(0)] + w_all(1, [0, 1]):
        cp.start()
    y_v[...] = jnp.zeros_like(y_v)
    hcol_v[pl.ds(F, FP - F), :] = jnp.zeros((FP - F, 128), f32)
    wd_v[pl.ds(F, FP - F), :] = jnp.zeros((FP - F, D), bf16)
    x_cp(0).wait()
    for cp in w_all(1, [2, 3]) + [x_cp(1)]:
        cp.start()
    zero = [pltpu.bitcast(y_v[:, 0:128], u32)]
    for w in prep_xs(0, 0, TH):
        w(None)
    for cp in w_all(1, [0]):
        cp.wait()
    for w in prep_ws(1, [0]):
        w(None)
    for cp in w_all(1, [1]):
        cp.wait()
    for (t, m), (fill, copies) in plan.items():
        k_finish(t, m, project(wks_v, (xa_v, xb_v)[t % 2], t // 2, m, fill, copies))
    for r in range(0, D, 8):
        zq_v[pl.ds(r // 16 * 16 + r // 8 % 2, 8, stride=2), :] = jnp.broadcast_to(
            jnp.sum(z_v[pl.ds(r, 8), :], axis=1, keepdims=True), (8, 128))

    wr = wr_ref[...].astype(f32).reshape(1, D)
    row8 = lax.broadcasted_iota(jnp.int32, (8, 1), 0)

    def q_tile(t, u, xs_v, top):
        def score(r0, n):
            base = pl.multiple_of(t * TS + r0, n)
            r = jnp.sum(bx_v[pl.ds(base, n), :].astype(f32) * wr, axis=1, keepdims=True)
            r = r.astype(bf16).astype(f32)
            for i in range(0, n, 8):
                upd = r[i:i + 8] > top[0]
                top[0] = jnp.where(upd, r[i:i + 8], top[0])
                top[1] = jnp.where(upd, row8 + (base + i), top[1])

        for m in range(NM):
            c = project(wqs_v, xs_v, u, m, [lambda v, r=r: score(r, 64) for r in range(m * TS // NM, (m + 1) * TS // NM, 64)])
            p = []
            for i, q in enumerate(c):
                pq = _phi(q)
                zc = zq_v[pl.ds((i // 2) * HD + m * MC, MC), :]
                zc = jnp.concatenate([zc] * (TH // 128), axis=1)
                den = jnp.sum((pq * zc).reshape(MC // DH, DH, TH), axis=1, keepdims=True) + 1e-6
                p.append((pq.reshape(MC // DH, DH, TH) * (1.0 / den)).reshape(MC, TH).T)
            for i, a in enumerate(_left(p[0], p[2], p[1], p[3])):
                qs_v[t, i, :, pl.ds(m * MC, MC)] = _pack(a)

    def q_body(u, carry):
        top = list(carry)
        b_cp(2 * u).wait()
        b_cp(2 * u + 1).wait()

        @pl.when(u == 0)
        def _():
            for j in range(1, NP):
                for i in range(2):
                    f_cp(j, i).start()

        @pl.when(u == 1)
        def _():
            for j in range(NP):
                f_cp(j, 2).start()

        q_tile(2 * u, u, xa_v, top)
        q_tile(2 * u + 1, u, xb_v, top)
        return tuple(top)

    best, bidx = lax.fori_loop(0, NT // 2, q_body, (jnp.full((8, 1), -jnp.inf, f32), row8))
    top_r = jnp.max(best)
    idx = jnp.min(jnp.where(best == top_r, bidx, S - 1))
    slab = pl.ds(pl.multiple_of((idx // 16) * 16, 16), 16)
    picked = lax.broadcasted_iota(jnp.int32, (16, D), 0) == idx % 16
    xsel = jnp.sum(jnp.where(picked, bx_v[slab, :].astype(f32), 0.0), axis=0, keepdims=True)
    xcol_v[...] = jnp.broadcast_to(xsel, (128, D)).T
    for g in range(2 * NP):
        v_cp(g).wait()
    wo_cp.wait()
    for j in range(NP):
        for i in range(2):
            f_cp(j, i).wait()

    def matvec(acc, w_ref, w0, col_ref, c0, n):
        for r in range(0, n, 16):
            w = w_ref[pl.ds(w0 + r, 16), :].astype(f32)
            pr = w * jnp.concatenate([col_ref[pl.ds(c0 + r, 16), :]] * (w.shape[1] // 128), axis=1)
            acc[0] = acc[0] + (pr[0:8] + pr[8:16])
        return acc[0]

    def before(words, fill):
        for w in fill:
            bits = pltpu.bitcast(w(), u32)
            dep = zero[0]
            for l in range(0, bits.shape[1], 128):
                dep = dep & bits[:, l:l + 128]
            top = words[0:8] | jnp.concatenate([dep] * (words.shape[1] // 128), axis=1)
            words = jnp.concatenate([top, words[8:]], axis=0)
        return words

    blk = (lax.broadcasted_iota(jnp.int32, (128, 128), 0) // DH) == (lax.broadcasted_iota(jnp.int32, (128, 128), 1) // DH)
    x_of = (0, 6, 1, 4, 5, 3, 2)

    def p_body(j, carry):
        ga, ua = [jnp.zeros((8, FC), f32)], [jnp.zeros((8, FC), f32)]
        fill = []
        for s in range(0, D, FR):
            fill.append(lambda s=s: matvec(ga, wg_v.at[j], s, xcol_v, s, FR))
            fill.append(lambda s=s: matvec(ua, wu_v.at[j], s, xcol_v, s, FR))
        rows = _half(j * 128, 128)

        def prod(i):
            acc = None
            for t in range(NT):
                k = i * NT + t
                lhs = before(ks_v[t, i, rows, :], fill[(k * len(fill)) // PK:((k + 1) * len(fill)) // PK])
                d = _dot(_unpack(lhs), _unpack((xa_v, xb_v)[t % 2][t // 2, x_of[i]]))
                acc = d if acc is None else acc + d
            return acc

        d11, d12, d21, d22 = _strassen(prod)
        g = jnp.sum(ga[0], axis=0, keepdims=True)
        u = jnp.sum(ua[0], axis=0, keepdims=True)
        hcol_v[pl.ds(pl.multiple_of(j * FC, 128), FC), :] = jnp.broadcast_to(g * _sigmoid(g) * u, (128, FC)).T
        for h, (lo, hi) in enumerate(((d11, d21), (d12, d22))):
            p_v[h, rows, :] = _pack(jnp.concatenate([lo, hi], axis=1))
        return carry

    lax.fori_loop(0, NP, p_body, 0)

    for j in range(NP):
        ms = []
        for h in (0, 1):
            grp = h * NP + j
            kv = _dot(_unpack(p_v[h, _half(j * 128, 128), :]), wv_v[grp])
            kv = jnp.where(blk, kv, 0.0).astype(bf16)
            mh = _dot(kv, wo_v[pl.ds(grp * 128, 128), :])
            ms += [mh[:, :HD], mh[:, HD:]]
        for i, b in enumerate(_right(*ms)):
            ms_v[i, _half(j * 128, 128), :] = _pack(b)

    gw = gw_ref[...].astype(f32).reshape(1, D)

    def o_body(step, carry):
        t = (idx // TS + 1 + step) % NT

        @pl.when(step == 0)
        def _():
            for j in range(NP):
                f_cp(j, 2).wait()

        @pl.when(step == NT - 1)
        def _():
            y = jnp.sum(y_v[...], axis=0, keepdims=True) * _sigmoid(jnp.full((1, D), top_r, f32))
            old = bx_v[slab, :].astype(f32)
            bx_v[slab, :] = jnp.where(picked, old + y, old).astype(bf16)

        r0 = pl.multiple_of(jnp.minimum(step, NT - 2) * FO, 16)
        ya = [y_v[...]]
        fill = [lambda s=s: matvec(ya, wd_v, r0 + s, hcol_v, r0 + s, DR) for s in range(0, FO, DR)]
        nprod = 7 * (TH // OC)
        for c in range(TH // OC):
            def prod(i):
                k = 7 * c + i
                lhs = before(qs_v[t, i, _half(c * OC, OC), :],
                             fill[(k * len(fill)) // nprod:((k + 1) * len(fill)) // nprod])
                return _dot(_unpack(lhs), _unpack(ms_v[i]))

            a = _strassen(prod)
            for h in (0, 1):
                rows = pl.ds(h * TH + c * OC, OC)
                g = _sigmoid(jnp.sum(x_v[t, rows, :].astype(f32) * gw, axis=1, keepdims=True))
                b = bx_v[pl.ds(pl.multiple_of(t * TS + h * TH + c * OC, OC), OC), :].astype(f32)
                ah = jnp.concatenate([a[2 * h], a[2 * h + 1]], axis=1)
                o_v[t, rows, :] = (g * ah + (1.0 - g) * b).astype(bf16)
                o_cp(t, h * (TH // OC) + c).start()
        y_v[...] = ya[0]
        return carry

    lax.fori_loop(0, NT, o_body, 0)
    for t in range(NT):
        for c in range(TS // OC):
            o_cp(t, c).wait()


@jax.jit
def pallas_gated_mix__linear_attn_block__moe_arch_mod__prompt_kernel(
        A_x, A_wqkv, A_wo, B_x, B_w_r, B_w_gate, B_w_up, B_w_down, gate_w):
    hbm = pl.BlockSpec(memory_space=pl.ANY)
    vmem = pl.BlockSpec(memory_space=pltpu.VMEM)
    return pl.pallas_call(
        _kernel,
        out_shape=jax.ShapeDtypeStruct((1, S, D), bf16),
        in_specs=[hbm, hbm, hbm, hbm, vmem, hbm, hbm, hbm, vmem],
        out_specs=hbm,
        scratch_shapes=[
            pltpu.VMEM((NT, TS, D), bf16),
            pltpu.VMEM((2, NP, 2, D, 128), bf16),
            pltpu.VMEM((2 * NP, D, 128), bf16),
            pltpu.VMEM((D, D), bf16),
            pltpu.VMEM((S, D), bf16),
            pltpu.VMEM((NP, D, FC), bf16),
            pltpu.VMEM((NP, D, FC), bf16),
            pltpu.VMEM((FP, D), bf16),
            pltpu.VMEM((NT // 2, 7, TH // 2, HD), u32),
            pltpu.VMEM((NT // 2, 7, TH // 2, HD), u32),
            pltpu.VMEM((7, HD // 2, HD), u32),
            pltpu.VMEM((7, HD // 2, HD), u32),
            pltpu.VMEM((NT, 7, HD // 2, TH), u32),
            pltpu.VMEM((NT, 7, TH // 2, HD), u32),
            pltpu.VMEM((2, HD // 2, D), u32),
            pltpu.VMEM((7, HD // 2, HD), u32),
            pltpu.VMEM((D, 128), f32),
            pltpu.VMEM((D, 128), f32),
            pltpu.VMEM((D, 128), f32),
            pltpu.VMEM((FP, 128), f32),
            pltpu.VMEM((8, D), f32),
            pltpu.VMEM((NT, TS, D), bf16),
            pltpu.SemaphoreType.DMA((NT,)),
            pltpu.SemaphoreType.DMA((4 * NP,)),
            pltpu.SemaphoreType.DMA((2 * NP + 1,)),
            pltpu.SemaphoreType.DMA((NT,)),
            pltpu.SemaphoreType.DMA((3 * NP,)),
            pltpu.SemaphoreType.DMA((S // OC,)),
        ],
        compiler_params=pltpu.CompilerParams(vmem_limit_bytes=110 * 1024 * 1024, flags=FLAGS),
    )(A_x, A_wqkv, A_wo, B_x, B_w_r, B_w_gate, B_w_up, B_w_down, gate_w)
```

```python
import jax
import jax.numpy as jnp
from jax import lax
import jax.experimental.pallas as pl
import jax.experimental.pallas.tpu as pltpu

S, D, F, DH = 2048, 1024, 3584, 32
TS = 512
TH = TS // 2
NT = S // TS
HD = D // 2
MC = 128
NM = HD // MC
NP = HD // 128
FC = F // NP
FO = 1200
FP = (NT - 1) * FO
DR = 48
PK = 28
PRE1, PRE2, PRE3 = [], [1, 2], [3]
FLAGS = None
FN = 7
FR = 128
OC = 64
f32, bf16, u32 = jnp.float32, jnp.bfloat16, jnp.uint32


def _phi(t):
    return jnp.maximum(t + 1e-6, 1e-6) + jnp.exp(jnp.minimum(t, 0.0))


def _sigmoid(t):
    return 1.0 / (1.0 + jnp.exp(-t))


def _dot(a, b):
    return jnp.dot(a, b, preferred_element_type=f32)


def _dot_nt(a, b):
    return lax.dot_general(a, b, (((1,), (1,)), ((), ())), preferred_element_type=f32)


def _pack(v):
    return pltpu.bitcast(v.astype(bf16), u32)


def _pack2(even, odd):
    return pltpu.pack_elementwise([even, odd], packed_dtype=bf16)


def _pack_mixed(v):
    r, c = v.shape
    v = v.reshape(r // 16, 2, 8, c)
    return _pack2(v[:, 0].reshape(r // 2, c), v[:, 1].reshape(r // 2, c))


def _unpack(w):
    return pltpu.bitcast(w, bf16)


def _half(start, size):
    if isinstance(start, int):
        return pl.ds(start // 2, size // 2)
    return pl.ds(pl.multiple_of(start // 2, size // 2), size // 2)


def _left(a11, a12, a21, a22):
    return (a11 + a22, a21 + a22, a11, a22, a11 + a12, a21 - a11, a12 - a22)


def _right(b11, b12, b21, b22):
    return (b11 + b22, b11, b12 - b22, b21 - b11, b22, b11 + b12, b21 + b22)


def _strassen(prod, work=()):
    m = []
    for i in range(7):
        m.append(prod(i))
        for at, w in work:
            if i <= 7 * at < i + 1:
                w(m[i])
    return (m[0] + m[3]) + (m[6] - m[4]), m[2] + m[4], m[1] + m[3], (m[0] - m[1]) + (m[2] + m[5])


def _spread(pieces, lo=0.0, hi=1.0):
    return [(lo + (hi - lo) * k / len(pieces), w) for k, w in enumerate(pieces)]


def _kernel(x_hbm, wqkv_hbm, wo_hbm, wr_hbm, wg_hbm, wu_hbm, wd_hbm, gw_hbm, out_hbm,
            x_v, wqk_v, wv_v, wo_v, wg_v, wu_v, wd_v,
            xa_v, xb_v, wqs_v, wks_v, ks_v, qs_v, p_v, ms_v, z_v, zq_v, xcol_v, hcol_v, y_v, o_v, wr_v, gw_v,
            sem_x, sem_w, sem_v, sem_f, sem_o):
    def x_cp(t):
        return pltpu.make_async_copy(x_hbm.at[0, pl.ds(t * TS, TS)], x_v.at[t], sem_x.at[t])

    def w_cp(j, m, h):
        return pltpu.make_async_copy(wqkv_hbm.at[:, pl.ds(j * D + h * HD + m * 128, 128)],
                                     wqk_v.at[j, m, h], sem_w.at[(j * NP + m) * 2 + h])

    def v_cp(g):
        return pltpu.make_async_copy(wqkv_hbm.at[:, pl.ds(2 * D + g * 128, 128)], wv_v.at[g], sem_v.at[g])

    wo_cp = pltpu.make_async_copy(wo_hbm, wo_v, sem_v.at[2 * NP])

    wr_cp = pltpu.make_async_copy(wr_hbm, wr_v, sem_v.at[2 * NP + 1])
    gw_cp = pltpu.make_async_copy(gw_hbm, gw_v, sem_v.at[2 * NP + 2])

    def f_cp(j, i):
        cols = pl.ds(j * FC, FC)
        if i == 2:
            return pltpu.make_async_copy(wd_hbm.at[cols], wd_v.at[cols], sem_f.at[i * NP + j])
        return pltpu.make_async_copy((wg_hbm, wu_hbm)[i].at[:, cols], (wg_v, wu_v)[i].at[j], sem_f.at[i * NP + j])

    def o_cp(t, c):
        return pltpu.make_async_copy(o_v.at[t, pl.ds(c * OC, OC)], out_hbm.at[0, pl.ds(t * TS + c * OC, OC)],
                                     sem_o.at[t * (TS // OC) + c])

    def after(words, v):
        if v is None:
            return words
        dep = zero[0] & pltpu.bitcast(v[0:8, 0:128], u32)
        r, c = words.shape
        return (words.reshape(r // 8, 8, c) | jnp.concatenate([dep] * (c // 128), axis=1)).reshape(r, c)

    def words_of(block, v):
        return after(pltpu.bitcast(block, u32), v)

    def prep_w(j, m, k, v):
        blk = [_unpack(words_of(wqk_v[j, m, h, pl.ds(i * HD + k * 128, 128), :], v)).astype(f32).T
               for h in (0, 1) for i in (0, 1)]
        for i, a in enumerate(_left(*blk)):
            (wqs_v, wks_v)[j][i, _half(m * 128, 128), pl.ds(k * 128, 128)] = (_pack_mixed, _pack)[j](a)

    def prep_x(src, dst_v, dst, r, n, v):
        blk = [words_of(x_v[src, pl.ds(h * TH + r, n), pl.ds(i * HD, HD)], v) for i in (0, 1) for h in (0, 1)]
        even, odd = (_right(*[pltpu.unpack_elementwise(b, index=p, packed_dtype=bf16, unpacked_dtype=f32)
                              for b in blk]) for p in (0, 1))
        for i in range(7):
            dst_v[dst, i, _half(r, n), :] = blk[0] if i == 1 else blk[3] if i == 4 else _pack2(even[i], odd[i])

    def project(w_v, xs_v, u, m, work):
        rows = _half(m * MC, MC)
        return _strassen(lambda i: _dot_nt(_unpack(w_v[i, rows, :]), _unpack(xs_v[u, i])), work)

    def w_all(j, ms):
        return [w_cp(j, m, h) for m in ms for h in (0, 1)]

    def prep_ws(j, ms):
        return [lambda v, m=m, k=k: prep_w(j, m, k, v) for m in ms for k in range(HD // 128)]

    def prep_xs(t, r0, r1):
        return [lambda v, r=r: prep_x(t, (xa_v, xb_v)[t % 2], t // 2, r, 16, v) for r in range(r0, r1, 16)]

    def k_finish(t, m, c):
        c11, c12, c21, c22 = [_phi(b) for b in c]
        for h, zs in enumerate((c11 + c12, c21 + c22)):
            zr = pl.ds(h * HD + m * MC, MC)
            zs = sum(zs[:, l:l + 128] for l in range(128, TH, 128)) + zs[:, 0:128]
            zs = zs if t == 0 else z_v[zr, :] + zs
            if t < NT - 1:
                z_v[zr, :] = zs
            else:
                zs = jnp.broadcast_to(jnp.sum(zs, axis=1, keepdims=True), (MC, 128))
                for r in range(0, MC, 8):
                    zq_v[pl.ds(h * HD + m * MC + r // 16 * 16 + r // 8 % 2, 8, stride=2), :] = zs[r:r + 8]
        for i, b in enumerate(_right(c11, c21, c12, c22)):
            ks_v[t, i, _half(m * MC, MC), :] = _pack_mixed(b)

    def sync(at, waits, starts):
        def run(_):
            for cp in waits:
                cp.wait()
            for cp in starts:
                cp.start()
        return [(at, run)]

    end = 0.8
    plan = {
        (0, 0): sync(0.15, w_all(1, [1]), [x_cp(1)]) + _spread(prep_ws(1, [1]), 0.15, end)
        + sync(end, w_all(1, [2]), []),
        (0, 1): _spread(prep_ws(1, [2]), 0, end) + sync(end, w_all(1, [3]), [x_cp(2)]),
        (0, 2): _spread(prep_ws(1, [3]), 0, 0.4) + sync(0.4, [x_cp(1)], w_all(0, [0, 1]))
        + _spread(prep_xs(1, 0, 96), 0.4),
        (0, 3): _spread(prep_xs(1, 96, TH), 0, end)
        + sync(end, [x_cp(2)], [x_cp(3)] + w_all(0, [2, 3])),
    }
    for m in range(NM):
        plan[1, m] = _spread(prep_xs(2, m * 64, m * 64 + 64), 0, end if m == NM - 1 else 1)
    plan[1, NM - 1] += sync(end, [x_cp(3)] + w_all(0, range(NP)),
                            [v_cp(g) for g in range(2 * NP)]
                            + [wo_cp, wr_cp, gw_cp, f_cp(0, 0), f_cp(0, 1)])
    for m in range(NM):
        plan[2, m] = _spread(prep_xs(3, m * 64, m * 64 + 64))
    for m in range(NM):
        plan[3, m] = _spread(prep_ws(0, [m]))

    for cp in [x_cp(0)] + w_all(1, [0]):
        cp.start()
    y_v[...] = jnp.zeros_like(y_v)
    hcol_v[pl.ds(F, FP - F), :] = jnp.zeros((FP - F, 128), f32)
    wd_v[pl.ds(F, FP - F), :] = jnp.zeros((FP - F, D), bf16)
    for cp in w_all(1, PRE1):
        cp.start()
    x_cp(0).wait()
    for cp in w_all(1, PRE2):
        cp.start()
    zero = [pltpu.bitcast(y_v[:, 0:128], u32)]
    for w in prep_xs(0, 0, TH):
        w(None)
    for cp in w_all(1, [0]):
        cp.wait()
    for cp in w_all(1, PRE3):
        cp.start()
    for w in prep_ws(1, [0]):
        w(None)
    for (t, m), work in plan.items():
        k_finish(t, m, project(wks_v, (xa_v, xb_v)[t % 2], t // 2, m, work))

    wr_cp.wait()
    wr = wr_v[...].astype(f32).reshape(1, D)
    row8 = lax.broadcasted_iota(jnp.int32, (8, 1), 0)

    def q_tile(t, u, xs_v, top):
        def score(r0, n):
            base = t * TS + r0
            r = jnp.sum(x_v[t, pl.ds(r0, n), :].astype(f32) * wr, axis=1, keepdims=True)
            r = r.astype(bf16).astype(f32)
            for i in range(0, n, 8):
                upd = r[i:i + 8] > top[0]
                top[0] = jnp.where(upd, r[i:i + 8], top[0])
                top[1] = jnp.where(upd, row8 + (base + i), top[1])

        for m in range(NM):
            c = project(wqs_v, xs_v, u, m, _spread(
                [lambda v, r=r: score(r, 64) for r in range(m * TS // NM, (m + 1) * TS // NM, 64)], 0.43))
            p = []
            for i, q in enumerate(c):
                pq = _phi(q)
                zc = zq_v[pl.ds((i // 2) * HD + m * MC, MC), :]
                zc = jnp.concatenate([zc] * (TH // 128), axis=1)
                den = jnp.sum((pq * zc).reshape(MC // DH, DH, TH), axis=1, keepdims=True) + 1e-6
                p.append((pq.reshape(MC // DH, DH, TH) * (1.0 / den)).reshape(MC, TH).T)
            for i, a in enumerate(_left(p[0], p[2], p[1], p[3])):
                qs_v[t, i, :, pl.ds(m * MC, MC)] = _pack(a)

    def q_body(u, carry):
        top = list(carry)

        @pl.when(u == 0)
        def _():
            for j in range(1, NP):
                for i in range(2):
                    f_cp(j, i).start()

        @pl.when(u == 1)
        def _():
            for j in range(NP):
                f_cp(j, 2).start()

        q_tile(2 * u, u, xa_v, top)
        q_tile(2 * u + 1, u, xb_v, top)
        return tuple(top)

    best, bidx = lax.fori_loop(0, NT // 2, q_body, (jnp.full((8, 1), -jnp.inf, f32), row8))
    top_r = jnp.max(best)
    idx = jnp.min(jnp.where(best == top_r, bidx, S - 1))
    slab = x_v[idx // TS, pl.ds(pl.multiple_of(idx % TS // 16 * 16, 16), 16), :].astype(f32)
    picked = lax.broadcasted_iota(jnp.int32, (16, D), 0) == idx % 16
    xsel = jnp.sum(jnp.where(picked, slab, 0.0), axis=0, keepdims=True)
    xcol_v[...] = jnp.broadcast_to(xsel, (128, D)).T
    for g in range(2 * NP):
        v_cp(g).wait()
    wo_cp.wait()
    gw_cp.wait()
    for j in range(NP):
        for i in range(2):
            f_cp(j, i).wait()

    def matvec(acc, w_ref, w0, col_ref, c0, n):
        for r in range(0, n, 16):
            w = w_ref[pl.ds(w0 + r, 16), :].astype(f32)
            pr = w * jnp.concatenate([col_ref[pl.ds(c0 + r, 16), :]] * (w.shape[1] // 128), axis=1)
            acc[0] = acc[0] + (pr[0:8] + pr[8:16])
        return acc[0]

    def before(words, fill):
        for w in fill:
            bits = pltpu.bitcast(w(), u32)
            dep = zero[0]
            for l in range(0, bits.shape[1], 128):
                dep = dep & bits[:, l:l + 128]
            top = words[0:8] | jnp.concatenate([dep] * (words.shape[1] // 128), axis=1)
            words = jnp.concatenate([top, words[8:]], axis=0)
        return words

    blk = (lax.broadcasted_iota(jnp.int32, (128, 128), 0) // DH) == (lax.broadcasted_iota(jnp.int32, (128, 128), 1) // DH)
    x_of = (0, 6, 1, 4, 5, 3, 2)

    def p_body(j, carry):
        ga, ua = [jnp.zeros((8, FC), f32)], [jnp.zeros((8, FC), f32)]
        fill = []
        for s in range(0, D, FR):
            fill.append(lambda s=s: matvec(ga, wg_v.at[j], s, xcol_v, s, FR))
            fill.append(lambda s=s: matvec(ua, wu_v.at[j], s, xcol_v, s, FR))
        rows = _half(j * 128, 128)

        def prod(i):
            acc = None
            for t in range(NT):
                k = i * NT + t
                lhs = before(ks_v[t, i, rows, :], fill[(k * len(fill)) // PK:((k + 1) * len(fill)) // PK])
                d = _dot(_unpack(lhs), _unpack((xa_v, xb_v)[t % 2][t // 2, x_of[i]]))
                acc = d if acc is None else acc + d
            return acc

        d11, d12, d21, d22 = _strassen(prod)
        g = jnp.sum(ga[0], axis=0, keepdims=True)
        u = jnp.sum(ua[0], axis=0, keepdims=True)
        hcol_v[pl.ds(pl.multiple_of(j * FC, 128), FC), :] = jnp.broadcast_to(g * _sigmoid(g) * u, (128, FC)).T
        for h, (lo, hi) in enumerate(((d11, d21), (d12, d22))):
            p_v[h, rows, :] = _pack(jnp.concatenate([lo, hi], axis=1))
        return carry

    lax.fori_loop(0, NP, p_body, 0)

    for j in range(NP):
        ms = []
        for h in (0, 1):
            grp = h * NP + j
            kv = _dot(_unpack(p_v[h, _half(j * 128, 128), :]), wv_v[grp])
            kv = jnp.where(blk, kv, 0.0).astype(bf16)
            mh = _dot(kv, wo_v[pl.ds(grp * 128, 128), :])
            ms += [mh[:, :HD], mh[:, HD:]]
        for i, b in enumerate(_right(*ms)):
            ms_v[i, _half(j * 128, 128), :] = _pack(b)

    gw = gw_v[...].astype(f32).reshape(1, D)

    def o_body(step, carry):
        t = (idx // TS + 1 + step) % NT

        @pl.when(step == 0)
        def _():
            for j in range(NP):
                f_cp(j, 2).wait()

        y = jnp.sum(y_v[...], axis=0, keepdims=True) * _sigmoid(jnp.full((1, D), top_r, f32))
        r0 = pl.multiple_of(jnp.minimum(step, NT - 2) * FO, 16)
        ya = [y_v[...]]
        fill = [lambda s=s: matvec(ya, wd_v, r0 + s, hcol_v, r0 + s, DR) for s in range(0, FO, DR)]
        nprod = 7 * (TH // OC)
        for c in range(TH // OC):
            def prod(i):
                k = 7 * c + i
                lhs = before(qs_v[t, i, _half(c * OC, OC), :],
                             fill[(k * len(fill)) // nprod:((k + 1) * len(fill)) // nprod])
                return _dot(_unpack(lhs), _unpack(ms_v[i]))

            a = _strassen(prod)
            for h in (0, 1):
                rows = pl.ds(h * TH + c * OC, OC)
                x = x_v[t, rows, :].astype(f32)
                g = _sigmoid(jnp.sum(x * gw, axis=1, keepdims=True))
                token = lax.broadcasted_iota(jnp.int32, (OC, D), 0) + (t * TS + h * TH + c * OC)
                b = jnp.where(token == idx, x + y, x)
                ah = jnp.concatenate([a[2 * h], a[2 * h + 1]], axis=1)
                o_v[t, rows, :] = (g * ah + (1.0 - g) * b).astype(bf16)
                o_cp(t, h * (TH // OC) + c).start()
        y_v[...] = ya[0]
        return carry

    lax.fori_loop(0, NT, o_body, 0)
    for t in range(NT):
        for c in range(TS // OC):
            o_cp(t, c).wait()


@jax.jit
def pallas_gated_mix__linear_attn_block__moe_arch_mod__prompt_kernel(
        A_x, A_wqkv, A_wo, B_x, B_w_r, B_w_gate, B_w_up, B_w_down, gate_w):
    del B_x
    hbm = pl.BlockSpec(memory_space=pl.ANY)
    return pl.pallas_call(
        _kernel,
        out_shape=jax.ShapeDtypeStruct((1, S, D), bf16),
        in_specs=[hbm] * 8,
        out_specs=hbm,
        scratch_shapes=[
            pltpu.VMEM((NT, TS, D), bf16),
            pltpu.VMEM((2, NP, 2, D, 128), bf16),
            pltpu.VMEM((2 * NP, D, 128), bf16),
            pltpu.VMEM((D, D), bf16),
            pltpu.VMEM((NP, D, FC), bf16),
            pltpu.VMEM((NP, D, FC), bf16),
            pltpu.VMEM((FP, D), bf16),
            pltpu.VMEM((NT // 2, 7, TH // 2, HD), u32),
            pltpu.VMEM((NT // 2, 7, TH // 2, HD), u32),
            pltpu.VMEM((7, HD // 2, HD), u32),
            pltpu.VMEM((7, HD // 2, HD), u32),
            pltpu.VMEM((NT, 7, HD // 2, TH), u32),
            pltpu.VMEM((NT, 7, TH // 2, HD), u32),
            pltpu.VMEM((2, HD // 2, D), u32),
            pltpu.VMEM((7, HD // 2, HD), u32),
            pltpu.VMEM((D, 128), f32),
            pltpu.VMEM((D, 128), f32),
            pltpu.VMEM((D, 128), f32),
            pltpu.VMEM((FP, 128), f32),
            pltpu.VMEM((8, D), f32),
            pltpu.VMEM((NT, TS, D), bf16),
            pltpu.VMEM((D,), bf16),
            pltpu.VMEM((D,), bf16),
            pltpu.SemaphoreType.DMA((NT,)),
            pltpu.SemaphoreType.DMA((4 * NP,)),
            pltpu.SemaphoreType.DMA((2 * NP + 3,)),
            pltpu.SemaphoreType.DMA((3 * NP,)),
            pltpu.SemaphoreType.DMA((S // OC,)),
        ],
        compiler_params=pltpu.CompilerParams(vmem_limit_bytes=110 * 1024 * 1024, flags=FLAGS),
    )(A_x, A_wqkv, A_wo, B_w_r, B_w_gate, B_w_up, B_w_down, gate_w)
```

```python
import jax
import jax.numpy as jnp
from jax import lax
import jax.experimental.pallas as pl
import jax.experimental.pallas.tpu as pltpu

S, D, F, DH = 2048, 1024, 3584, 32
TS = 512
TH = TS // 2
NT = S // TS
HD = D // 2
MC = 128
NM = HD // MC
NP = HD // 128
FC = F // NP
FO = 1200
FP = (NT - 1) * FO
DR = 48
PK = 26
KT = True
XR = 16
END = 0.65
RM = 1
PRE1, PRE2, PRE3 = [], [1, 2], [3]
FLAGS = None
FN = 7
FR = 64
OC = 64
f32, bf16, u32 = jnp.float32, jnp.bfloat16, jnp.uint32


def _phi(t):
    return jnp.maximum(t + 1e-6, 1e-6) + jnp.exp(jnp.minimum(t, 0.0))


def _sigmoid(t):
    return 1.0 / (1.0 + jnp.exp(-t))


def _dot(a, b):
    return jnp.dot(a, b, preferred_element_type=f32)


def _dot_nt(a, b):
    return lax.dot_general(a, b, (((1,), (1,)), ((), ())), preferred_element_type=f32)


def _pack(v):
    return pltpu.bitcast(v.astype(bf16), u32)


def _pack2(even, odd):
    return pltpu.pack_elementwise([even, odd], packed_dtype=bf16)


def _pack_mixed(v):
    r, c = v.shape
    v = v.reshape(r // 16, 2, 8, c)
    return _pack2(v[:, 0].reshape(r // 2, c), v[:, 1].reshape(r // 2, c))


def _unpack(w):
    return pltpu.bitcast(w, bf16)


def _half(start, size):
    if isinstance(start, int):
        return pl.ds(start // 2, size // 2)
    return pl.ds(pl.multiple_of(start // 2, size // 2), size // 2)


def _left(a11, a12, a21, a22):
    return (a11 + a22, a21 + a22, a11, a22, a11 + a12, a21 - a11, a12 - a22)


def _right(b11, b12, b21, b22):
    return (b11 + b22, b11, b12 - b22, b21 - b11, b22, b11 + b12, b21 + b22)


def _strassen(prod, work=()):
    m = []
    for i in range(7):
        m.append(prod(i))
        for at, w in work:
            if i <= 7 * at < i + 1:
                w(m[i])
    return (m[0] + m[3]) + (m[6] - m[4]), m[2] + m[4], m[1] + m[3], (m[0] - m[1]) + (m[2] + m[5])


def _spread(pieces, lo=0.0, hi=1.0):
    return [(lo + (hi - lo) * k / len(pieces), w) for k, w in enumerate(pieces)]


def _kernel(x_hbm, wqkv_hbm, wo_hbm, wr_hbm, wg_hbm, wu_hbm, wd_hbm, gw_hbm, out_hbm,
            x_v, wqk_v, wv_v, wo_v, wg_v, wu_v, wd_v,
            xa_v, xb_v, wqs_v, wks_v, ks_v, qs_v, p_v, ms_v, z_v, zq_v, xcol_v, hcol_v, y_v, o_v, wr_v, gw_v,
            sem_x, sem_w, sem_v, sem_f, sem_o):
    def x_cp(t):
        return pltpu.make_async_copy(x_hbm.at[0, pl.ds(t * TS, TS)], x_v.at[t], sem_x.at[t])

    def w_cp(j, m, h):
        return pltpu.make_async_copy(wqkv_hbm.at[:, pl.ds(j * D + h * HD + m * 128, 128)],
                                     wqk_v.at[j, m, h], sem_w.at[(j * NP + m) * 2 + h])

    def v_cp(g):
        return pltpu.make_async_copy(wqkv_hbm.at[:, pl.ds(2 * D + g * 128, 128)], wv_v.at[g], sem_v.at[g])

    wo_cp = pltpu.make_async_copy(wo_hbm, wo_v, sem_v.at[2 * NP])

    wr_cp = pltpu.make_async_copy(wr_hbm, wr_v, sem_v.at[2 * NP + 1])
    gw_cp = pltpu.make_async_copy(gw_hbm, gw_v, sem_v.at[2 * NP + 2])

    def f_cp(j, i):
        cols = pl.ds(j * FC, FC)
        if i == 2:
            return pltpu.make_async_copy(wd_hbm.at[cols], wd_v.at[cols], sem_f.at[i * NP + j])
        return pltpu.make_async_copy((wg_hbm, wu_hbm)[i].at[:, cols], (wg_v, wu_v)[i].at[j], sem_f.at[i * NP + j])

    def o_cp(t, c):
        return pltpu.make_async_copy(o_v.at[t, pl.ds(c * OC, OC)], out_hbm.at[0, pl.ds(t * TS + c * OC, OC)],
                                     sem_o.at[t * (TS // OC) + c])

    def after(words, v):
        if v is None or not KT:
            return words
        dep = zero[0] & pltpu.bitcast(v[0:8, 0:128], u32)
        r, c = words.shape
        return (words.reshape(r // 8, 8, c) | jnp.concatenate([dep] * (c // 128), axis=1)).reshape(r, c)

    def words_of(block, v):
        return after(pltpu.bitcast(block, u32), v)

    def prep_w(j, m, k, v):
        blk = [_unpack(words_of(wqk_v[j, m, h, pl.ds(i * HD + k * 128, 128), :], v)).astype(f32).T
               for h in (0, 1) for i in (0, 1)]
        for i, a in enumerate(_left(*blk)):
            (wqs_v, wks_v)[j][i, _half(m * 128, 128), pl.ds(k * 128, 128)] = (_pack, _pack_mixed)[j](a)

    def prep_x(src, dst_v, dst, r, n, v):
        blk = [words_of(x_v[src, pl.ds(h * TH + r, n), pl.ds(i * HD, HD)], v) for i in (0, 1) for h in (0, 1)]
        vals = [[pltpu.unpack_elementwise(b, index=p, packed_dtype=bf16, unpacked_dtype=f32) for b in blk]
                for p in (0, 1)]
        even, odd = _right(*vals[0]), _right(*vals[1])
        for p in (0, 1):
            for h in (0, 1):
                score = jnp.sum(vals[p][h] * top[2][:, :HD] + vals[p][2 + h] * top[2][:, HD:], axis=1, keepdims=True)
                score = score.astype(bf16).astype(f32)
                token = 2 * row8 + (src * TS + h * TH + r + p)
                better = (score > top[0]) | ((score == top[0]) & (token < top[1]))
                top[0], top[1] = jnp.where(better, score, top[0]), jnp.where(better, token, top[1])
        for i in range(7):
            dst_v[dst, i, _half(r, n), :] = blk[0] if i == 1 else blk[3] if i == 4 else _pack2(even[i], odd[i])

    def project(w_v, xs_v, u, m, work):
        rows = _half(m * MC, MC)
        return _strassen(lambda i: _dot_nt(_unpack(w_v[i, rows, :]), _unpack(xs_v[u, i])), work)

    def w_all(j, ms):
        return [w_cp(j, m, h) for m in ms for h in (0, 1)]

    def prep_ws(j, ms):
        return [lambda v, m=m, k=k: prep_w(j, m, k, v) for m in ms for k in range(HD // 128)]

    def prep_xs(t, r0, r1):
        return [lambda v, r=r: prep_x(t, (xa_v, xb_v)[t % 2], t // 2, r, XR, v) for r in range(r0, r1, XR)]

    def k_finish(t, m, c):
        c11, c12, c21, c22 = [_phi(b) for b in c]
        for h, zs in enumerate((c11 + c12, c21 + c22)):
            zr = pl.ds(h * HD + m * MC, MC)
            zs = sum(zs[:, l:l + 128] for l in range(128, TH, 128)) + zs[:, 0:128]
            zs = zs if t == 0 else z_v[zr, :] + zs
            if t < NT - 1:
                z_v[zr, :] = zs
            else:
                z_v[zr, :] = jnp.broadcast_to(jnp.sum(zs, axis=1, keepdims=True), (MC, 128))
                for r in range(h * HD + m * MC, h * HD + (m + 1) * MC, 8):
                    zq_v[pl.ds(r, 8), :] = z_v[pl.ds(r // 16 * 16 + r // 8 % 2, 8, stride=2), :]
        for i, b in enumerate(_right(c11, c21, c12, c22)):
            ks_v[t, i, _half(m * MC, MC), :] = _pack_mixed(b)

    row8 = lax.broadcasted_iota(jnp.int32, (8, 1), 0)
    top = [jnp.full((8, 1), -jnp.inf, f32), row8, None]

    def route(_):
        best = jnp.max(top[0])
        idx = jnp.min(jnp.where(top[0] == best, top[1], S - 1))
        top[0], top[1] = best, idx
        slab = x_v[idx // TS, pl.ds(pl.multiple_of(idx % TS // 16 * 16, 16), 16), :].astype(f32)
        picked = lax.broadcasted_iota(jnp.int32, (16, D), 0) == idx % 16
        xcol_v[...] = jnp.broadcast_to(jnp.sum(jnp.where(picked, slab, 0.0), axis=0, keepdims=True), (128, D)).T

    def sync(at, waits, starts):
        def run(_):
            for cp in waits:
                cp.wait()
            for cp in starts:
                cp.start()
        return [(at, run)]

    end = END
    plan = {
        (0, 0): sync(0.15, w_all(1, [1]), [x_cp(1)]) + _spread(prep_ws(1, [1]), 0.15, end)
        + sync(end, w_all(1, [2]), []),
        (0, 1): _spread(prep_ws(1, [2]), 0, end) + sync(end, w_all(1, [3]), [x_cp(2)]),
        (0, 2): _spread(prep_ws(1, [3]), 0, 0.4) + sync(0.4, [x_cp(1)], w_all(0, [0, 1]))
        + _spread(prep_xs(1, 0, 96), 0.4),
        (0, 3): _spread(prep_xs(1, 96, TH), 0, end)
        + sync(end, [x_cp(2)], [x_cp(3)] + w_all(0, [2, 3])),
    }
    for m in range(NM):
        plan[1, m] = _spread(prep_xs(2, m * 64, m * 64 + 64), 0, end if m == NM - 1 else 1)
    plan[1, NM - 1] += sync(end, [x_cp(3)] + w_all(0, range(NP)),
                            [v_cp(g) for g in range(2 * NP)]
                            + [wo_cp, gw_cp, f_cp(0, 0), f_cp(0, 1)])
    for m in range(NM):
        plan[2, m] = _spread(prep_xs(3, m * 64, m * 64 + 64))
    for m in range(NM):
        plan[3, m] = _spread(prep_ws(0, [m]))
    plan[3, RM].append((0.5, route))

    for cp in [wr_cp, x_cp(0)] + w_all(1, [0]):
        cp.start()
    y_v[...] = jnp.zeros_like(y_v)
    hcol_v[pl.ds(F, FP - F), :] = jnp.zeros((FP - F, 128), f32)
    wd_v[pl.ds(F, FP - F), :] = jnp.zeros((FP - F, D), bf16)
    zero = [pltpu.bitcast(y_v[:, 0:128], u32)]
    for cp in w_all(1, [0]):
        cp.wait()
    for cp in w_all(1, PRE1):
        cp.start()
    for w in prep_ws(1, [0]):
        w(None)
    wr_cp.wait()
    top[2] = wr_v[...].astype(f32).reshape(1, D)
    x_cp(0).wait()
    for cp in w_all(1, PRE2):
        cp.start()
    for w in prep_xs(0, 0, TH):
        w(None)
    for cp in w_all(1, PRE3):
        cp.start()
    for (t, m), work in plan.items():
        k_finish(t, m, project(wks_v, (xa_v, xb_v)[t % 2], t // 2, m, work))

    top_r, idx = top[:2]

    def q_tile(t, u, xs_v):
        for m in range(NM):
            c = project(wqs_v, xs_v, u, m, [])
            p = []
            for i, q in enumerate(c):
                pq = _phi(q)
                zc = zq_v[pl.ds((i // 2) * HD + m * MC, MC), :]
                zc = jnp.concatenate([zc] * (TH // 128), axis=1)
                den = jnp.sum((pq * zc).reshape(MC // DH, DH, TH), axis=1, keepdims=True) + 1e-6
                p.append((pq.reshape(MC // DH, DH, TH) * (1.0 / den)).reshape(MC, TH).T)
            for i, a in enumerate(_left(p[0], p[2], p[1], p[3])):
                qs_v[t, i, :, pl.ds(m * MC, MC)] = _pack(a)

    def q_body(u, carry):

        @pl.when(u == 0)
        def _():
            for j in range(1, NP):
                for i in range(2):
                    f_cp(j, i).start()

        @pl.when(u == 1)
        def _():
            for j in range(NP):
                f_cp(j, 2).start()

        q_tile(2 * u, u, xa_v)
        q_tile(2 * u + 1, u, xb_v)
        return carry

    lax.fori_loop(0, NT // 2, q_body, 0)
    for g in range(2 * NP):
        v_cp(g).wait()
    wo_cp.wait()
    gw_cp.wait()
    for j in range(NP):
        for i in range(2):
            f_cp(j, i).wait()

    def matvec(acc, w_ref, w0, col_ref, c0, n):
        for r in range(0, n, 16):
            w = w_ref[pl.ds(w0 + r, 16), :].astype(f32)
            pr = w * jnp.concatenate([col_ref[pl.ds(c0 + r, 16), :]] * (w.shape[1] // 128), axis=1)
            acc[0] = acc[0] + (pr[0:8] + pr[8:16])
        return acc[0]

    def before(words, fill):
        for w in fill:
            bits = pltpu.bitcast(w(), u32)
            dep = zero[0]
            for l in range(0, bits.shape[1], 128):
                dep = dep & bits[:, l:l + 128]
            top = words[0:8] | jnp.concatenate([dep] * (words.shape[1] // 128), axis=1)
            words = jnp.concatenate([top, words[8:]], axis=0)
        return words

    blk = (lax.broadcasted_iota(jnp.int32, (128, 128), 0) // DH) == (lax.broadcasted_iota(jnp.int32, (128, 128), 1) // DH)
    x_of = (0, 6, 1, 4, 5, 3, 2)

    def p_body(j, carry):
        ga, ua = [jnp.zeros((8, FC), f32)], [jnp.zeros((8, FC), f32)]
        fill = []
        for s in range(0, D, FR):
            fill.append(lambda s=s: matvec(ga, wg_v.at[j], s, xcol_v, s, FR))
            fill.append(lambda s=s: matvec(ua, wu_v.at[j], s, xcol_v, s, FR))
        rows = _half(j * 128, 128)

        def prod(i):
            acc = None
            for t in range(NT):
                k = i * NT + t
                lhs = before(ks_v[t, i, rows, :], fill[(k * len(fill)) // PK:((k + 1) * len(fill)) // PK])
                d = _dot(_unpack(lhs), _unpack((xa_v, xb_v)[t % 2][t // 2, x_of[i]]))
                acc = d if acc is None else acc + d
            return acc

        d11, d12, d21, d22 = _strassen(prod)
        g = jnp.sum(ga[0], axis=0, keepdims=True)
        u = jnp.sum(ua[0], axis=0, keepdims=True)
        hcol_v[pl.ds(pl.multiple_of(j * FC, 128), FC), :] = jnp.broadcast_to(g * _sigmoid(g) * u, (128, FC)).T
        for h, (lo, hi) in enumerate(((d11, d21), (d12, d22))):
            p_v[h, rows, :] = _pack_mixed(jnp.concatenate([lo, hi], axis=1))
        return carry

    lax.fori_loop(0, NP, p_body, 0)

    for j in range(NP):
        ms = []
        for h in (0, 1):
            grp = h * NP + j
            kv = _dot(_unpack(p_v[h, _half(j * 128, 128), :]), wv_v[grp])
            kv = jnp.where(blk, kv, 0.0).astype(bf16)
            mh = _dot(kv, wo_v[pl.ds(grp * 128, 128), :])
            ms += [mh[:, :HD], mh[:, HD:]]
        for i, b in enumerate(_right(*ms)):
            ms_v[i, _half(j * 128, 128), :] = _pack_mixed(b)

    gw = gw_v[...].astype(f32).reshape(1, D)

    def o_body(step, carry):
        t = (idx // TS + 1 + step) % NT

        @pl.when(step == 0)
        def _():
            for j in range(NP):
                f_cp(j, 2).wait()

        y = jnp.sum(y_v[...], axis=0, keepdims=True) * _sigmoid(jnp.full((1, D), top_r, f32))
        r0 = pl.multiple_of(jnp.minimum(step, NT - 2) * FO, 16)
        ya = [y_v[...]]
        fill = [lambda s=s: matvec(ya, wd_v, r0 + s, hcol_v, r0 + s, DR) for s in range(0, FO, DR)]
        nprod = 7 * (TH // OC)
        for c in range(TH // OC):
            def prod(i):
                k = 7 * c + i
                lhs = before(qs_v[t, i, _half(c * OC, OC), :],
                             fill[(k * len(fill)) // nprod:((k + 1) * len(fill)) // nprod])
                return _dot(_unpack(lhs), _unpack(ms_v[i]))

            a = _strassen(prod)
            for h in (0, 1):
                rows = pl.ds(h * TH + c * OC, OC)
                x = x_v[t, rows, :].astype(f32)
                g = _sigmoid(jnp.sum(x * gw, axis=1, keepdims=True))
                token = lax.broadcasted_iota(jnp.int32, (OC, D), 0) + (t * TS + h * TH + c * OC)
                b = jnp.where(token == idx, x + y, x)
                ah = jnp.concatenate([a[2 * h], a[2 * h + 1]], axis=1)
                o_v[t, rows, :] = (g * ah + (1.0 - g) * b).astype(bf16)
                o_cp(t, h * (TH // OC) + c).start()
        y_v[...] = ya[0]
        return carry

    lax.fori_loop(0, NT, o_body, 0)
    for t in range(NT):
        for c in range(TS // OC):
            o_cp(t, c).wait()


@jax.jit
def pallas_gated_mix__linear_attn_block__moe_arch_mod__prompt_kernel(
        A_x, A_wqkv, A_wo, B_x, B_w_r, B_w_gate, B_w_up, B_w_down, gate_w):
    del B_x
    hbm = pl.BlockSpec(memory_space=pl.ANY)
    return pl.pallas_call(
        _kernel,
        out_shape=jax.ShapeDtypeStruct((1, S, D), bf16),
        in_specs=[hbm] * 8,
        out_specs=hbm,
        scratch_shapes=[
            pltpu.VMEM((NT, TS, D), bf16),
            pltpu.VMEM((2, NP, 2, D, 128), bf16),
            pltpu.VMEM((2 * NP, D, 128), bf16),
            pltpu.VMEM((D, D), bf16),
            pltpu.VMEM((NP, D, FC), bf16),
            pltpu.VMEM((NP, D, FC), bf16),
            pltpu.VMEM((FP, D), bf16),
            pltpu.VMEM((NT // 2, 7, TH // 2, HD), u32),
            pltpu.VMEM((NT // 2, 7, TH // 2, HD), u32),
            pltpu.VMEM((7, HD // 2, HD), u32),
            pltpu.VMEM((7, HD // 2, HD), u32),
            pltpu.VMEM((NT, 7, HD // 2, TH), u32),
            pltpu.VMEM((NT, 7, TH // 2, HD), u32),
            pltpu.VMEM((2, HD // 2, D), u32),
            pltpu.VMEM((7, HD // 2, HD), u32),
            pltpu.VMEM((D + 8, 128), f32),
            pltpu.VMEM((D, 128), f32),
            pltpu.VMEM((D, 128), f32),
            pltpu.VMEM((FP, 128), f32),
            pltpu.VMEM((8, D), f32),
            pltpu.VMEM((NT, TS, D), bf16),
            pltpu.VMEM((D,), bf16),
            pltpu.VMEM((D,), bf16),
            pltpu.SemaphoreType.DMA((NT,)),
            pltpu.SemaphoreType.DMA((4 * NP,)),
            pltpu.SemaphoreType.DMA((2 * NP + 3,)),
            pltpu.SemaphoreType.DMA((3 * NP,)),
            pltpu.SemaphoreType.DMA((S // OC,)),
        ],
        compiler_params=pltpu.CompilerParams(vmem_limit_bytes=110 * 1024 * 1024, flags=FLAGS),
    )(A_x, A_wqkv, A_wo, B_w_r, B_w_gate, B_w_up, B_w_down, gate_w)
```

```python
import jax
import jax.numpy as jnp
from jax import lax
import jax.experimental.pallas as pl
import jax.experimental.pallas.tpu as pltpu

S, D, F, DH = 2048, 1024, 3584, 32
TS = 512
TH = TS // 2
NT = S // TS
HD = D // 2
MC = 128
NM = HD // MC
FC = F // NM
FR = 64
PK = 26
OC = 64
FO = 1200
FP = (NT - 1) * FO
DR = 48
f32, bf16, u32 = jnp.float32, jnp.bfloat16, jnp.uint32


def _phi(t):
    return jnp.maximum(t + 1e-6, 1e-6) + jnp.exp(jnp.minimum(t, 0.0))


def _sigmoid(t):
    return 1.0 / (1.0 + jnp.exp(-t))


def _dot(a, b):
    return jnp.dot(a, b, preferred_element_type=f32)


def _dot_nt(a, b):
    return lax.dot_general(a, b, (((1,), (1,)), ((), ())), preferred_element_type=f32)


def _pack(v):
    return pltpu.bitcast(v.astype(bf16), u32)


def _pack2(even, odd):
    return pltpu.pack_elementwise([even, odd], packed_dtype=bf16)


def _pack_mixed(v):
    r, c = v.shape
    v = v.reshape(r // 16, 2, 8, c)
    return _pack2(v[:, 0].reshape(r // 2, c), v[:, 1].reshape(r // 2, c))


def _unpack(w):
    return pltpu.bitcast(w, bf16)


def _half(start, size):
    if isinstance(start, int):
        return pl.ds(start // 2, size // 2)
    return pl.ds(pl.multiple_of(start // 2, size // 2), size // 2)


def _left(a11, a12, a21, a22):
    return (a11 + a22, a21 + a22, a11, a22, a11 + a12, a21 - a11, a12 - a22)


def _right(b11, b12, b21, b22):
    return (b11 + b22, b11, b12 - b22, b21 - b11, b22, b11 + b12, b21 + b22)


def _strassen(prod, work=()):
    m = []
    for i in range(7):
        m.append(prod(i))
        for at, w in work:
            if i <= 7 * at < i + 1:
                w(m[i])
    return (m[0] + m[3]) + (m[6] - m[4]), m[2] + m[4], m[1] + m[3], (m[0] - m[1]) + (m[2] + m[5])


def _spread(pieces, lo=0.0, hi=1.0):
    return [(lo + (hi - lo) * k / len(pieces), w) for k, w in enumerate(pieces)]


def _kernel(x_hbm, wqkv_hbm, wo_hbm, wr_hbm, wg_hbm, wu_hbm, wd_hbm, gw_hbm, out_hbm,
            x_v, wqk_v, wv_v, wo_v, wg_v, wu_v, wd_v,
            xa_v, xb_v, wqs_v, wks_v, ks_v, qs_v, p_v, ms_v, z_v, kv_v, xcol_v, hcol_v, y_v, o_v, wr_v, gw_v,
            sem_x, sem_w, sem_v, sem_f, sem_o):
    def x_cp(t):
        return pltpu.make_async_copy(x_hbm.at[0, pl.ds(t * TS, TS)], x_v.at[t], sem_x.at[t])

    def w_cp(j, m, h):
        return pltpu.make_async_copy(wqkv_hbm.at[:, pl.ds(j * D + h * HD + m * 128, 128)],
                                     wqk_v.at[j, m, h], sem_w.at[(j * NM + m) * 2 + h])

    def v_cp(g):
        return pltpu.make_async_copy(wqkv_hbm.at[:, pl.ds(2 * D + g * 128, 128)], wv_v.at[g], sem_v.at[g])

    wo_cp = pltpu.make_async_copy(wo_hbm, wo_v, sem_v.at[2 * NM])

    wr_cp = pltpu.make_async_copy(wr_hbm, wr_v, sem_v.at[2 * NM + 1])
    gw_cp = pltpu.make_async_copy(gw_hbm, gw_v, sem_v.at[2 * NM + 2])

    def f_cp(j, i):
        cols = pl.ds(j * FC, FC)
        if i == 2:
            return pltpu.make_async_copy(wd_hbm.at[cols], wd_v.at[cols], sem_f.at[i * NM + j])
        return pltpu.make_async_copy((wg_hbm, wu_hbm)[i].at[:, cols], (wg_v, wu_v)[i].at[j], sem_f.at[i * NM + j])

    def o_cp(t, c):
        return pltpu.make_async_copy(o_v.at[t, pl.ds(c * OC, OC)], out_hbm.at[0, pl.ds(t * TS + c * OC, OC)],
                                     sem_o.at[t * (TS // OC) + c])

    def after(words, v):
        if v is None:
            return words
        dep = zero[0] & pltpu.bitcast(v[0:8, 0:128], u32)
        r, c = words.shape
        return (words.reshape(r // 8, 8, c) | jnp.concatenate([dep] * (c // 128), axis=1)).reshape(r, c)

    def words_of(block, v):
        return after(pltpu.bitcast(block, u32), v)

    def prep_w(j, m, k, v):
        blk = [_unpack(words_of(wqk_v[j, m, h, pl.ds(i * HD + k * 128, 128), :], v)).astype(f32).T
               for h in (0, 1) for i in (0, 1)]
        for i, a in enumerate(_left(*blk)):
            (wqs_v, wks_v)[j][i, _half(m * 128, 128), pl.ds(k * 128, 128)] = _pack_mixed(a)

    def prep_x(src, dst_v, dst, r, n, v):
        blk = [words_of(x_v[src, pl.ds(h * TH + r, n), pl.ds(i * HD, HD)], v) for i in (0, 1) for h in (0, 1)]
        vals = [[pltpu.unpack_elementwise(b, index=p, packed_dtype=bf16, unpacked_dtype=f32) for b in blk]
                for p in (0, 1)]
        even, odd = _right(*vals[0]), _right(*vals[1])
        for p in (0, 1):
            for h in (0, 1):
                score = jnp.sum(vals[p][h] * top[2][:, :HD] + vals[p][2 + h] * top[2][:, HD:], axis=1, keepdims=True)
                score = score.astype(bf16).astype(f32)
                token = 2 * row8 + (src * TS + h * TH + r + p)
                better = (score > top[0]) | ((score == top[0]) & (token < top[1]))
                top[0], top[1] = jnp.where(better, score, top[0]), jnp.where(better, token, top[1])
        for i in range(7):
            dst_v[dst, i, _half(r, n), :] = blk[0] if i == 1 else blk[3] if i == 4 else _pack2(even[i], odd[i])

    def project(w_v, xs_v, u, m, work):
        rows = _half(m * MC, MC)
        return _strassen(lambda i: _dot_nt(_unpack(w_v[i, rows, :]), _unpack(xs_v[u, i])), work)

    def w_all(j, ms):
        return [w_cp(j, m, h) for m in ms for h in (0, 1)]

    def prep_ws(j, ms):
        return [lambda v, m=m, k=k: prep_w(j, m, k, v) for m in ms for k in range(HD // 128)]

    def prep_xs(t, r0, r1):
        return [lambda v, r=r: prep_x(t, (xa_v, xb_v)[t % 2], t // 2, r, 16, v) for r in range(r0, r1, 16)]

    def k_finish(t, m, c):
        c11, c12, c21, c22 = [_phi(b) for b in c]
        for h, zs in enumerate((c11 + c12, c21 + c22)):
            zr = pl.ds(h * HD + m * MC, MC)
            zs = sum(zs[:, l:l + 128] for l in range(128, TH, 128)) + zs[:, 0:128]
            zs = zs if t == 0 else z_v[zr, :] + zs
            if t == NT - 1:
                zs = jnp.broadcast_to(jnp.sum(zs, axis=1, keepdims=True), (MC, 128))
            z_v[zr, :] = zs
        for i, b in enumerate(_right(c11, c21, c12, c22)):
            ks_v[t, i, _half(m * MC, MC), :] = _pack_mixed(b)

    row8 = lax.broadcasted_iota(jnp.int32, (8, 1), 0)
    top = [jnp.full((8, 1), -jnp.inf, f32), row8, None]

    def route(_):
        best = jnp.max(top[0])
        idx = jnp.min(jnp.where(top[0] == best, top[1], S - 1))
        top[0], top[1] = best, idx
        slab = x_v[idx // TS, pl.ds(pl.multiple_of(idx % TS // 16 * 16, 16), 16), :].astype(f32)
        picked = lax.broadcasted_iota(jnp.int32, (16, D), 0) == idx % 16
        xcol_v[...] = jnp.broadcast_to(jnp.sum(jnp.where(picked, slab, 0.0), axis=0, keepdims=True), (128, D)).T

    def sync(at, waits, starts):
        def run(_):
            for cp in waits:
                cp.wait()
            for cp in starts:
                cp.start()
        return [(at, run)]

    end = 0.65
    plan = {
        (0, 0): sync(0.15, w_all(1, [1]), [x_cp(1)]) + _spread(prep_ws(1, [1]), 0.15, end)
        + sync(end, w_all(1, [2]), []),
        (0, 1): _spread(prep_ws(1, [2]), 0, end) + sync(end, w_all(1, [3]), [x_cp(2)]),
        (0, 2): _spread(prep_ws(1, [3]), 0, 0.4) + sync(0.4, [x_cp(1)], w_all(0, [0, 1]))
        + _spread(prep_xs(1, 0, 96), 0.4),
        (0, 3): _spread(prep_xs(1, 96, TH), 0, end)
        + sync(end, [x_cp(2)], [x_cp(3)] + w_all(0, [2, 3])),
    }
    for m in range(NM):
        plan[1, m] = _spread(prep_xs(2, m * 64, m * 64 + 64), 0, end if m == NM - 1 else 1)
    plan[1, NM - 1] += sync(end, [x_cp(3)] + w_all(0, range(NM)),
                            [v_cp(g) for g in range(2 * NM)]
                            + [wo_cp, gw_cp, f_cp(0, 0), f_cp(0, 1)])
    for m in range(NM):
        plan[2, m] = _spread(prep_xs(3, m * 64, m * 64 + 64))
    for m in range(NM):
        plan[3, m] = _spread(prep_ws(0, [m]))
    plan[3, 2].append((0.5, route))

    for cp in [wr_cp, x_cp(0)] + w_all(1, [0]):
        cp.start()
    y_v[...] = jnp.zeros_like(y_v)
    hcol_v[pl.ds(F, FP - F), :] = jnp.zeros((FP - F, 128), f32)
    wd_v[pl.ds(F, FP - F), :] = jnp.zeros((FP - F, D), bf16)
    zero = [pltpu.bitcast(y_v[:, 0:128], u32)]
    for cp in w_all(1, [0]):
        cp.wait()
    for w in prep_ws(1, [0]):
        w(None)
    wr_cp.wait()
    top[2] = wr_v[...].astype(f32).reshape(1, D)
    x_cp(0).wait()
    for cp in w_all(1, [1, 2]):
        cp.start()
    for w in prep_xs(0, 0, TH):
        w(None)
    for cp in w_all(1, [3]):
        cp.start()
    for (t, m), work in plan.items():
        k_finish(t, m, project(wks_v, (xa_v, xb_v)[t % 2], t // 2, m, work))

    top_r, idx = top[:2]

    def q_tile(t, u, xs_v):
        for m in range(NM):
            c = project(wqs_v, xs_v, u, m, [])
            p = []
            for i, q in enumerate(c):
                pq = _phi(q)
                zc = z_v[pl.ds((i // 2) * HD + m * MC, MC), :]
                zc = jnp.concatenate([zc] * (TH // 128), axis=1)
                den = jnp.sum((pq * zc).reshape(MC // DH, DH, TH), axis=1, keepdims=True) + 1e-6
                p.append((pq.reshape(MC // DH, DH, TH) * (1.0 / den)).reshape(MC, TH).T)
            for i, a in enumerate(_left(p[0], p[2], p[1], p[3])):
                qs_v[t, i, :, pl.ds(m * MC, MC)] = _pack(a)

    def q_body(u, carry):

        @pl.when(u == 0)
        def _():
            for j in range(1, NM):
                for i in range(2):
                    f_cp(j, i).start()

        @pl.when(u == 1)
        def _():
            for j in range(NM):
                f_cp(j, 2).start()

        q_tile(2 * u, u, xa_v)
        q_tile(2 * u + 1, u, xb_v)
        return carry

    lax.fori_loop(0, NT // 2, q_body, 0)
    for g in range(2 * NM):
        v_cp(g).wait()
    wo_cp.wait()
    gw_cp.wait()
    for j in range(NM):
        for i in range(2):
            f_cp(j, i).wait()

    def matvec(acc, w_ref, w0, col_ref, c0, n):
        for r in range(0, n, 16):
            w = w_ref[pl.ds(w0 + r, 16), :].astype(f32)
            pr = w * jnp.concatenate([col_ref[pl.ds(c0 + r, 16), :]] * (w.shape[1] // 128), axis=1)
            acc[0] = acc[0] + (pr[0:8] + pr[8:16])
        return acc[0]

    def before(words, fill):
        for w in fill:
            bits = pltpu.bitcast(w(), u32)
            dep = zero[0]
            for l in range(0, bits.shape[1], 128):
                dep = dep & bits[:, l:l + 128]
            top = words[0:8] | jnp.concatenate([dep] * (words.shape[1] // 128), axis=1)
            words = jnp.concatenate([top, words[8:]], axis=0)
        return words

    blk = (lax.broadcasted_iota(jnp.int32, (128, 128), 0) // DH) == (lax.broadcasted_iota(jnp.int32, (128, 128), 1) // DH)
    x_of = (0, 6, 1, 4, 5, 3, 2)

    def p_body(j, carry):
        ga, ua = [jnp.zeros((8, FC), f32)], [jnp.zeros((8, FC), f32)]
        fill = []
        for s in range(0, D, FR):
            fill.append(lambda s=s: matvec(ga, wg_v.at[j], s, xcol_v, s, FR))
            fill.append(lambda s=s: matvec(ua, wu_v.at[j], s, xcol_v, s, FR))
        rows = _half(j * 128, 128)

        def prod(i):
            acc = None
            for t in range(NT):
                k = i * NT + t
                lhs = before(ks_v[t, i, rows, :], fill[(k * len(fill)) // PK:((k + 1) * len(fill)) // PK])
                d = _dot(_unpack(lhs), _unpack((xa_v, xb_v)[t % 2][t // 2, x_of[i]]))
                acc = d if acc is None else acc + d
            return acc

        d11, d12, d21, d22 = _strassen(prod)
        g = jnp.sum(ga[0], axis=0, keepdims=True)
        u = jnp.sum(ua[0], axis=0, keepdims=True)
        hcol_v[pl.ds(pl.multiple_of(j * FC, 128), FC), :] = jnp.broadcast_to(g * _sigmoid(g) * u, (128, FC)).T
        for h, (lo, hi) in enumerate(((d11, d21), (d12, d22))):
            p_v[h, rows, :] = _pack_mixed(jnp.concatenate([lo, hi], axis=1))
        return carry

    lax.fori_loop(0, NM, p_body, 0)

    for j in range(NM):
        ms = []
        for h in (0, 1):
            grp = h * NM + j
            kv = _dot(_unpack(p_v[h, _half(j * 128, 128), :]), wv_v[grp])
            kv = jnp.where(blk, kv, 0.0)
            for r in range(0, 128, 8):
                kv_v[pl.ds(grp * 128 + r // 16 * 16 + r // 8 % 2, 8, stride=2), :] = kv[r:r + 8]
            kv = kv_v[pl.ds(grp * 128, 128), :].astype(bf16)
            mh = _dot(kv, wo_v[pl.ds(grp * 128, 128), :])
            ms += [mh[:, :HD], mh[:, HD:]]
        for i, b in enumerate(_right(*ms)):
            ms_v[i, _half(j * 128, 128), :] = _pack_mixed(b)

    gw = gw_v[...].astype(f32).reshape(1, D)

    def o_body(step, carry):
        t = (idx // TS + 1 + step) % NT

        @pl.when(step == 0)
        def _():
            for j in range(NM):
                f_cp(j, 2).wait()

        y = jnp.sum(y_v[...], axis=0, keepdims=True) * _sigmoid(jnp.full((1, D), top_r, f32))
        r0 = pl.multiple_of(jnp.minimum(step, NT - 2) * FO, 16)
        ya = [y_v[...]]
        fill = [lambda s=s: matvec(ya, wd_v, r0 + s, hcol_v, r0 + s, DR) for s in range(0, FO, DR)]
        nprod = 7 * (TH // OC)
        for c in range(TH // OC):
            def prod(i):
                k = 7 * c + i
                lhs = before(qs_v[t, i, _half(c * OC, OC), :],
                             fill[(k * len(fill)) // nprod:((k + 1) * len(fill)) // nprod])
                return _dot(_unpack(lhs), _unpack(ms_v[i]))

            a = _strassen(prod)
            for h in (0, 1):
                rows = pl.ds(h * TH + c * OC, OC)
                x = x_v[t, rows, :].astype(f32)
                g = _sigmoid(jnp.sum(x * gw, axis=1, keepdims=True))
                token = lax.broadcasted_iota(jnp.int32, (OC, D), 0) + (t * TS + h * TH + c * OC)
                b = jnp.where(token == idx, x + y, x)
                ah = jnp.concatenate([a[2 * h], a[2 * h + 1]], axis=1)
                o_v[t, rows, :] = (g * ah + (1.0 - g) * b).astype(bf16)
                o_cp(t, h * (TH // OC) + c).start()
        y_v[...] = ya[0]
        return carry

    lax.fori_loop(0, NT, o_body, 0)
    for t in range(NT):
        for c in range(TS // OC):
            o_cp(t, c).wait()


@jax.jit
def pallas_gated_mix__linear_attn_block__moe_arch_mod__prompt_kernel(
        A_x, A_wqkv, A_wo, B_x, B_w_r, B_w_gate, B_w_up, B_w_down, gate_w):
    del B_x
    hbm = pl.BlockSpec(memory_space=pl.ANY)
    return pl.pallas_call(
        _kernel,
        out_shape=jax.ShapeDtypeStruct((1, S, D), bf16),
        in_specs=[hbm] * 8,
        out_specs=hbm,
        scratch_shapes=[
            pltpu.VMEM((NT, TS, D), bf16),
            pltpu.VMEM((2, NM, 2, D, 128), bf16),
            pltpu.VMEM((2 * NM, D, 128), bf16),
            pltpu.VMEM((D, D), bf16),
            pltpu.VMEM((NM, D, FC), bf16),
            pltpu.VMEM((NM, D, FC), bf16),
            pltpu.VMEM((FP, D), bf16),
            pltpu.VMEM((NT // 2, 7, TH // 2, HD), u32),
            pltpu.VMEM((NT // 2, 7, TH // 2, HD), u32),
            pltpu.VMEM((7, HD // 2, HD), u32),
            pltpu.VMEM((7, HD // 2, HD), u32),
            pltpu.VMEM((NT, 7, HD // 2, TH), u32),
            pltpu.VMEM((NT, 7, TH // 2, HD), u32),
            pltpu.VMEM((2, HD // 2, D), u32),
            pltpu.VMEM((7, HD // 2, HD), u32),
            pltpu.VMEM((D, 128), f32),
            pltpu.VMEM((D + 8, 128), f32),
            pltpu.VMEM((D, 128), f32),
            pltpu.VMEM((FP, 128), f32),
            pltpu.VMEM((8, D), f32),
            pltpu.VMEM((NT, TS, D), bf16),
            pltpu.VMEM((D,), bf16),
            pltpu.VMEM((D,), bf16),
            pltpu.SemaphoreType.DMA((NT,)),
            pltpu.SemaphoreType.DMA((4 * NM,)),
            pltpu.SemaphoreType.DMA((2 * NM + 3,)),
            pltpu.SemaphoreType.DMA((3 * NM,)),
            pltpu.SemaphoreType.DMA((S // OC,)),
        ],
        compiler_params=pltpu.CompilerParams(vmem_limit_bytes=110 * 1024 * 1024),
    )(A_x, A_wqkv, A_wo, B_w_r, B_w_gate, B_w_up, B_w_down, gate_w)
```

```python
import jax
import jax.numpy as jnp
from jax import lax
import jax.experimental.pallas as pl
import jax.experimental.pallas.tpu as pltpu

S, D, F, DH = 2048, 1024, 3584, 32
TS = 512
TH = TS // 2
NT = S // TS
HD = D // 2
MC = 128
NM = HD // MC
FC = F // NM
FR = 64
PK = 26
OC = 64
FO = 1200
FP = (NT - 1) * FO
DR = 48
f32, bf16, u32 = jnp.float32, jnp.bfloat16, jnp.uint32


def _phi(t):
    return jnp.maximum(t + 1e-6, 1e-6) + jnp.exp(jnp.minimum(t, 0.0))


def _sigmoid(t):
    return 1.0 / (1.0 + jnp.exp(-t))


def _dot(a, b):
    return jnp.dot(a, b, preferred_element_type=f32)


def _dot_nt(a, b):
    return lax.dot_general(a, b, (((1,), (1,)), ((), ())), preferred_element_type=f32)


def _pack(v):
    return pltpu.bitcast(v.astype(bf16), u32)


def _pack2(even, odd):
    return pltpu.pack_elementwise([even, odd], packed_dtype=bf16)


def _pack_mixed(v):
    r, c = v.shape
    v = v.reshape(r // 16, 2, 8, c)
    return _pack2(v[:, 0].reshape(r // 2, c), v[:, 1].reshape(r // 2, c))


def _unpack(w):
    return pltpu.bitcast(w, bf16)


def _half(start, size):
    if isinstance(start, int):
        return pl.ds(start // 2, size // 2)
    return pl.ds(pl.multiple_of(start // 2, size // 2), size // 2)


def _left(a11, a12, a21, a22):
    return (a11 + a22, a21 + a22, a11, a22, a11 + a12, a21 - a11, a12 - a22)


def _right(b11, b12, b21, b22):
    return (b11 + b22, b11, b12 - b22, b21 - b11, b22, b11 + b12, b21 + b22)


def _strassen(prod, work=()):
    m = []
    for i in range(7):
        m.append(prod(i))
        for at, w in work:
            if i <= 7 * at < i + 1:
                w(m[i])
    return (m[0] + m[3]) + (m[6] - m[4]), m[2] + m[4], m[1] + m[3], (m[0] - m[1]) + (m[2] + m[5])


def _spread(pieces, lo=0.0, hi=1.0):
    return [(lo + (hi - lo) * k / len(pieces), w) for k, w in enumerate(pieces)]


def _kernel(x_hbm, wqkv_hbm, wo_hbm, wr_hbm, wg_hbm, wu_hbm, wd_hbm, gw_hbm, out_hbm,
            x_v, wqk_v, wv_v, wo_v, wg_v, wu_v, wd_v,
            xa_v, xb_v, wqs_v, wks_v, ks_v, qs_v, p_v, ms_v, z_v, kv_v, xcol_v, hcol_v, y_v, o_v, wr_v, gw_v,
            sem_x, sem_w, sem_v, sem_f, sem_o):
    def x_cp(t):
        return pltpu.make_async_copy(x_hbm.at[0, pl.ds(t * TS, TS)], x_v.at[t], sem_x.at[t])

    def w_cp(j, m, h):
        return pltpu.make_async_copy(wqkv_hbm.at[:, pl.ds(j * D + h * HD + m * 128, 128)],
                                     wqk_v.at[j, m, h], sem_w.at[(j * NM + m) * 2 + h])

    def v_cp(g):
        return pltpu.make_async_copy(wqkv_hbm.at[:, pl.ds(2 * D + g * 128, 128)], wv_v.at[g], sem_v.at[g])

    wo_cp = pltpu.make_async_copy(wo_hbm, wo_v, sem_v.at[2 * NM])

    wr_cp = pltpu.make_async_copy(wr_hbm, wr_v, sem_v.at[2 * NM + 1])
    gw_cp = pltpu.make_async_copy(gw_hbm, gw_v, sem_v.at[2 * NM + 2])

    def f_cp(j, i):
        cols = pl.ds(j * FC, FC)
        if i == 2:
            return pltpu.make_async_copy(wd_hbm.at[cols], wd_v.at[cols], sem_f.at[i * NM + j])
        return pltpu.make_async_copy((wg_hbm, wu_hbm)[i].at[:, cols], (wg_v, wu_v)[i].at[j], sem_f.at[i * NM + j])

    def o_cp(t, c):
        return pltpu.make_async_copy(o_v.at[t, pl.ds(c * OC, OC)], out_hbm.at[0, pl.ds(t * TS + c * OC, OC)],
                                     sem_o.at[t * (TS // OC) + c])

    def after(words, v):
        if v is None:
            return words
        dep = zero[0] & pltpu.bitcast(v[0:8, 0:128], u32)
        r, c = words.shape
        return (words.reshape(r // 8, 8, c) | jnp.concatenate([dep] * (c // 128), axis=1)).reshape(r, c)

    def words_of(block, v):
        return after(pltpu.bitcast(block, u32), v)

    def prep_w(j, m, k, v):
        blk = [_unpack(words_of(wqk_v[j, m, h, pl.ds(i * HD + k * 128, 128), :], v)).astype(f32).T
               for h in (0, 1) for i in (0, 1)]
        for i, a in enumerate(_left(*blk)):
            (wqs_v, wks_v)[j][i, _half(m * 128, 128), pl.ds(k * 128, 128)] = _pack_mixed(a)

    def prep_x(src, dst_v, dst, r, n, v):
        blk = [words_of(x_v[src, pl.ds(h * TH + r, n), pl.ds(i * HD, HD)], v) for i in (0, 1) for h in (0, 1)]
        vals = [[pltpu.unpack_elementwise(b, index=p, packed_dtype=bf16, unpacked_dtype=f32) for b in blk]
                for p in (0, 1)]
        even, odd = _right(*vals[0]), _right(*vals[1])
        for p in (0, 1):
            for h in (0, 1):
                score = jnp.sum(vals[p][h] * top[2][:, :HD] + vals[p][2 + h] * top[2][:, HD:], axis=1, keepdims=True)
                score = score.astype(bf16).astype(f32)
                token = 2 * row8 + (src * TS + h * TH + r + p)
                better = (score > top[0]) | ((score == top[0]) & (token < top[1]))
                top[0], top[1] = jnp.where(better, score, top[0]), jnp.where(better, token, top[1])
        for i in range(7):
            dst_v[dst, i, _half(r, n), :] = blk[0] if i == 1 else blk[3] if i == 4 else _pack2(even[i], odd[i])

    def project(w_v, xs_v, u, m, work):
        rows = _half(m * MC, MC)
        return _strassen(lambda i: _dot_nt(_unpack(w_v[i, rows, :]), _unpack(xs_v[u, i])), work)

    def w_all(j, ms):
        return [w_cp(j, m, h) for m in ms for h in (0, 1)]

    def prep_ws(j, ms):
        return [lambda v, m=m, k=k: prep_w(j, m, k, v) for m in ms for k in range(HD // 128)]

    def prep_xs(t, r0, r1):
        return [lambda v, r=r: prep_x(t, (xa_v, xb_v)[t % 2], t // 2, r, 16, v) for r in range(r0, r1, 16)]

    def k_finish(t, m, c):
        c11, c12, c21, c22 = [_phi(b) for b in c]
        for h, zs in enumerate((c11 + c12, c21 + c22)):
            zr = pl.ds(h * HD + m * MC, MC)
            zs = sum(zs[:, l:l + 128] for l in range(128, TH, 128)) + zs[:, 0:128]
            zs = zs if t == 0 else z_v[zr, :] + zs
            if t == NT - 1:
                zs = jnp.broadcast_to(jnp.sum(zs, axis=1, keepdims=True), (MC, 128))
            z_v[zr, :] = zs
        for i, b in enumerate(_right(c11, c21, c12, c22)):
            ks_v[t, i, _half(m * MC, MC), :] = _pack_mixed(b)

    row8 = lax.broadcasted_iota(jnp.int32, (8, 1), 0)
    top = [jnp.full((8, 1), -jnp.inf, f32), row8, None]

    def route(_):
        best = jnp.max(top[0])
        idx = jnp.min(jnp.where(top[0] == best, top[1], S - 1))
        top[0], top[1] = best, idx
        slab = x_v[idx // TS, pl.ds(pl.multiple_of(idx % TS // 16 * 16, 16), 16), :].astype(f32)
        picked = lax.broadcasted_iota(jnp.int32, (16, D), 0) == idx % 16
        xcol_v[...] = jnp.broadcast_to(jnp.sum(jnp.where(picked, slab, 0.0), axis=0, keepdims=True), (128, D)).T

    def sync(at, waits, starts):
        def run(_):
            for cp in waits:
                cp.wait()
            for cp in starts:
                cp.start()
        return [(at, run)]

    early, end = 0.58, 0.65
    plan = {
        (0, 0): sync(0.15, w_all(1, [1]), [x_cp(1)]) + _spread(prep_ws(1, [1]), 0.15, end)
        + sync(end, w_all(1, [2]), []),
        (0, 1): _spread(prep_ws(1, [2]), 0, end) + sync(end, w_all(1, [3]), [x_cp(2)]),
        (0, 2): _spread(prep_ws(1, [3]), 0, 0.4) + sync(0.4, [x_cp(1)], w_all(0, [0, 1]))
        + _spread(prep_xs(1, 0, 96), 0.4),
        (0, 3): _spread(prep_xs(1, 96, TH), 0, end)
        + sync(end, [x_cp(2)], [x_cp(3)] + w_all(0, [2, 3])),
    }
    for m in range(NM):
        plan[1, m] = _spread(prep_xs(2, m * 64, m * 64 + 64), 0, early)
    plan[1, NM - 1] += sync(end, [x_cp(3)] + w_all(0, range(NM)),
                            [v_cp(g) for g in range(2 * NM)]
                            + [wo_cp, gw_cp, f_cp(0, 0), f_cp(0, 1)])
    for m in range(NM):
        plan[2, m] = _spread(prep_xs(3, m * 64, m * 64 + 64), 0, early)
    for m in range(NM):
        plan[3, m] = _spread(prep_ws(0, [m]), 0, early)
    plan[3, 2].append((0.5, route))

    for cp in [wr_cp, x_cp(0)] + w_all(1, [0]):
        cp.start()
    y_v[...] = jnp.zeros_like(y_v)
    hcol_v[pl.ds(F, FP - F), :] = jnp.zeros((FP - F, 128), f32)
    wd_v[pl.ds(F, FP - F), :] = jnp.zeros((FP - F, D), bf16)
    zero = [pltpu.bitcast(y_v[:, 0:128], u32)]
    for cp in w_all(1, [0]):
        cp.wait()
    for w in prep_ws(1, [0]):
        w(None)
    wr_cp.wait()
    top[2] = wr_v[...].astype(f32).reshape(1, D)
    x_cp(0).wait()
    for cp in w_all(1, [1, 2]):
        cp.start()
    for w in prep_xs(0, 0, TH):
        w(None)
    for cp in w_all(1, [3]):
        cp.start()
    for (t, m), work in plan.items():
        k_finish(t, m, project(wks_v, (xa_v, xb_v)[t % 2], t // 2, m, work))

    top_r, idx = top[:2]

    def q_tile(t, u, xs_v):
        for m in range(NM):
            c = project(wqs_v, xs_v, u, m, [])
            p = []
            for i, q in enumerate(c):
                pq = _phi(q)
                zc = z_v[pl.ds((i // 2) * HD + m * MC, MC), :]
                zc = jnp.concatenate([zc] * (TH // 128), axis=1)
                den = jnp.sum((pq * zc).reshape(MC // DH, DH, TH), axis=1, keepdims=True) + 1e-6
                p.append((pq.reshape(MC // DH, DH, TH) * (1.0 / den)).reshape(MC, TH).T)
            for i, a in enumerate(_left(p[0], p[2], p[1], p[3])):
                qs_v[t, i, :, pl.ds(m * MC, MC)] = _pack(a)

    def q_body(u, carry):

        @pl.when(u == 0)
        def _():
            for j in range(1, NM):
                for i in range(2):
                    f_cp(j, i).start()

        @pl.when(u == 1)
        def _():
            for j in range(NM):
                f_cp(j, 2).start()

        q_tile(2 * u, u, xa_v)
        q_tile(2 * u + 1, u, xb_v)
        return carry

    lax.fori_loop(0, NT // 2, q_body, 0)
    for g in range(2 * NM):
        v_cp(g).wait()
    wo_cp.wait()
    gw_cp.wait()
    for j in range(NM):
        for i in range(2):
            f_cp(j, i).wait()

    def matvec(acc, w_ref, w0, col_ref, c0, n):
        for r in range(0, n, 16):
            w = w_ref[pl.ds(w0 + r, 16), :].astype(f32)
            pr = w * jnp.concatenate([col_ref[pl.ds(c0 + r, 16), :]] * (w.shape[1] // 128), axis=1)
            acc[0] = acc[0] + (pr[0:8] + pr[8:16])
        return acc[0]

    def before(words, fill):
        for w in fill:
            bits = pltpu.bitcast(w(), u32)
            dep = zero[0]
            for l in range(0, bits.shape[1], 128):
                dep = dep & bits[:, l:l + 128]
            top = words[0:8] | jnp.concatenate([dep] * (words.shape[1] // 128), axis=1)
            words = jnp.concatenate([top, words[8:]], axis=0)
        return words

    blk = (lax.broadcasted_iota(jnp.int32, (128, 128), 0) // DH) == (lax.broadcasted_iota(jnp.int32, (128, 128), 1) // DH)
    x_of = (0, 6, 1, 4, 5, 3, 2)

    def p_body(j, carry):
        ga, ua = [jnp.zeros((8, FC), f32)], [jnp.zeros((8, FC), f32)]
        fill = []
        for s in range(0, D, FR):
            fill.append(lambda s=s: matvec(ga, wg_v.at[j], s, xcol_v, s, FR))
            fill.append(lambda s=s: matvec(ua, wu_v.at[j], s, xcol_v, s, FR))
        rows = _half(j * 128, 128)

        def prod(i):
            acc = None
            for t in range(NT):
                k = i * NT + t
                lhs = before(ks_v[t, i, rows, :], fill[(k * len(fill)) // PK:((k + 1) * len(fill)) // PK])
                d = _dot(_unpack(lhs), _unpack((xa_v, xb_v)[t % 2][t // 2, x_of[i]]))
                acc = d if acc is None else acc + d
            return acc

        d11, d12, d21, d22 = _strassen(prod)
        g = jnp.sum(ga[0], axis=0, keepdims=True)
        u = jnp.sum(ua[0], axis=0, keepdims=True)
        hcol_v[pl.ds(pl.multiple_of(j * FC, 128), FC), :] = jnp.broadcast_to(g * _sigmoid(g) * u, (128, FC)).T
        for h, (lo, hi) in enumerate(((d11, d21), (d12, d22))):
            p_v[h, rows, :] = _pack_mixed(jnp.concatenate([lo, hi], axis=1))
        return carry

    lax.fori_loop(0, NM, p_body, 0)

    for j in range(NM):
        ms = []
        for h in (0, 1):
            grp = h * NM + j
            kv = _dot(_unpack(p_v[h, _half(j * 128, 128), :]), wv_v[grp])
            kv = jnp.where(blk, kv, 0.0)
            for r in range(0, 128, 8):
                kv_v[pl.ds(grp * 128 + r // 16 * 16 + r // 8 % 2, 8, stride=2), :] = kv[r:r + 8]
            kv = kv_v[pl.ds(grp * 128, 128), :].astype(bf16)
            mh = _dot(kv, wo_v[pl.ds(grp * 128, 128), :])
            ms += [mh[:, :HD], mh[:, HD:]]
        for i, b in enumerate(_right(*ms)):
            ms_v[i, _half(j * 128, 128), :] = _pack_mixed(b)

    gw = gw_v[...].astype(f32).reshape(1, D)

    def o_body(step, carry):
        t = (idx // TS + 1 + step) % NT

        @pl.when(step == 0)
        def _():
            for j in range(NM):
                f_cp(j, 2).wait()

        y = jnp.sum(y_v[...], axis=0, keepdims=True) * _sigmoid(jnp.full((1, D), top_r, f32))
        r0 = pl.multiple_of(jnp.minimum(step, NT - 2) * FO, 16)
        ya = [y_v[...]]
        fill = [lambda s=s: matvec(ya, wd_v, r0 + s, hcol_v, r0 + s, DR) for s in range(0, FO, DR)]
        nprod = 7 * (TH // OC)
        for c in range(TH // OC):
            def prod(i):
                k = 7 * c + i
                lhs = before(qs_v[t, i, _half(c * OC, OC), :],
                             fill[(k * len(fill)) // nprod:((k + 1) * len(fill)) // nprod])
                return _dot(_unpack(lhs), _unpack(ms_v[i]))

            a = _strassen(prod)
            for h in (0, 1):
                rows = pl.ds(h * TH + c * OC, OC)
                x = x_v[t, rows, :].astype(f32)
                g = _sigmoid(jnp.sum(x * gw, axis=1, keepdims=True))
                token = lax.broadcasted_iota(jnp.int32, (OC, D), 0) + (t * TS + h * TH + c * OC)
                b = jnp.where(token == idx, x + y, x)
                ah = jnp.concatenate([a[2 * h], a[2 * h + 1]], axis=1)
                o_v[t, rows, :] = (g * ah + (1.0 - g) * b).astype(bf16)
                o_cp(t, h * (TH // OC) + c).start()
        y_v[...] = ya[0]
        return carry

    lax.fori_loop(0, NT, o_body, 0)
    for t in range(NT):
        for c in range(TS // OC):
            o_cp(t, c).wait()


@jax.jit
def pallas_gated_mix__linear_attn_block__moe_arch_mod__prompt_kernel(
        A_x, A_wqkv, A_wo, B_x, B_w_r, B_w_gate, B_w_up, B_w_down, gate_w):
    del B_x
    hbm = pl.BlockSpec(memory_space=pl.ANY)
    return pl.pallas_call(
        _kernel,
        out_shape=jax.ShapeDtypeStruct((1, S, D), bf16),
        in_specs=[hbm] * 8,
        out_specs=hbm,
        scratch_shapes=[
            pltpu.VMEM((NT, TS, D), bf16),
            pltpu.VMEM((2, NM, 2, D, 128), bf16),
            pltpu.VMEM((2 * NM, D, 128), bf16),
            pltpu.VMEM((D, D), bf16),
            pltpu.VMEM((NM, D, FC), bf16),
            pltpu.VMEM((NM, D, FC), bf16),
            pltpu.VMEM((FP, D), bf16),
            pltpu.VMEM((NT // 2, 7, TH // 2, HD), u32),
            pltpu.VMEM((NT // 2, 7, TH // 2, HD), u32),
            pltpu.VMEM((7, HD // 2, HD), u32),
            pltpu.VMEM((7, HD // 2, HD), u32),
            pltpu.VMEM((NT, 7, HD // 2, TH), u32),
            pltpu.VMEM((NT, 7, TH // 2, HD), u32),
            pltpu.VMEM((2, HD // 2, D), u32),
            pltpu.VMEM((7, HD // 2, HD), u32),
            pltpu.VMEM((D, 128), f32),
            pltpu.VMEM((D + 8, 128), f32),
            pltpu.VMEM((D, 128), f32),
            pltpu.VMEM((FP, 128), f32),
            pltpu.VMEM((8, D), f32),
            pltpu.VMEM((NT, TS, D), bf16),
            pltpu.VMEM((D,), bf16),
            pltpu.VMEM((D,), bf16),
            pltpu.SemaphoreType.DMA((NT,)),
            pltpu.SemaphoreType.DMA((4 * NM,)),
            pltpu.SemaphoreType.DMA((2 * NM + 3,)),
            pltpu.SemaphoreType.DMA((3 * NM,)),
            pltpu.SemaphoreType.DMA((S // OC,)),
        ],
        compiler_params=pltpu.CompilerParams(vmem_limit_bytes=110 * 1024 * 1024),
    )(A_x, A_wqkv, A_wo, B_w_r, B_w_gate, B_w_up, B_w_down, gate_w)
```

```python
import jax
import jax.numpy as jnp
from jax import lax
import jax.experimental.pallas as pl
import jax.experimental.pallas.tpu as pltpu

S, D, F, DH = 2048, 1024, 3584, 32
TS = 512
TH = TS // 2
NT = S // TS
HD = D // 2
MC = 128
NM = HD // MC
FC = F // NM
FR = 64
PK = 26
OC = 64
FO = 1200
FP = (NT - 1) * FO
DR = 48
f32, bf16, u32 = jnp.float32, jnp.bfloat16, jnp.uint32


def _phi(t):
    return jnp.maximum(t + 1e-6, 1e-6) + jnp.exp(jnp.minimum(t, 0.0))


def _sigmoid(t):
    return 1.0 / (1.0 + jnp.exp(-t))


def _dot(a, b):
    return jnp.dot(a, b, preferred_element_type=f32)


def _dot_nt(a, b):
    return lax.dot_general(a, b, (((1,), (1,)), ((), ())), preferred_element_type=f32)


def _pack(v):
    return pltpu.bitcast(v.astype(bf16), u32)


def _pack2(even, odd):
    return pltpu.pack_elementwise([even, odd], packed_dtype=bf16)


def _pack_mixed(v):
    r, c = v.shape
    v = v.reshape(r // 16, 2, 8, c)
    return _pack2(v[:, 0].reshape(r // 2, c), v[:, 1].reshape(r // 2, c))


def _unpack(w):
    return pltpu.bitcast(w, bf16)


def _half(start, size):
    if isinstance(start, int):
        return pl.ds(start // 2, size // 2)
    return pl.ds(pl.multiple_of(start // 2, size // 2), size // 2)


def _left(a11, a12, a21, a22):
    return (a11 + a22, a21 + a22, a11, a22, a11 + a12, a21 - a11, a12 - a22)


def _right(b11, b12, b21, b22):
    return (b11 + b22, b11, b12 - b22, b21 - b11, b22, b11 + b12, b21 + b22)


def _strassen(prod, work=()):
    m = []
    for i in range(7):
        m.append(prod(i))
        for at, w in work:
            if i <= 7 * at < i + 1:
                w(m[i])
    return (m[0] + m[3]) + (m[6] - m[4]), m[2] + m[4], m[1] + m[3], (m[0] - m[1]) + (m[2] + m[5])


def _spread(pieces, lo=0.0, hi=1.0):
    return [(lo + (hi - lo) * k / len(pieces), w) for k, w in enumerate(pieces)]


def _kernel(x_hbm, wqkv_hbm, wo_hbm, wr_hbm, wg_hbm, wu_hbm, wd_hbm, gw_hbm, out_hbm,
            x_v, wqk_v, wv_v, wo_v, wg_v, wu_v, wd_v,
            xa_v, xb_v, wqs_v, wks_v, ks_v, qs_v, p_v, ms_v, z_v, kv_v, xcol_v, hcol_v, y_v, o_v, wr_v, gw_v,
            sem_x, sem_w, sem_v, sem_f, sem_o):
    def x_cp(t):
        return pltpu.make_async_copy(x_hbm.at[0, pl.ds(t * TS, TS)], x_v.at[t], sem_x.at[t])

    def w_cp(j, m, h):
        return pltpu.make_async_copy(wqkv_hbm.at[:, pl.ds(j * D + h * HD + m * 128, 128)],
                                     wqk_v.at[j, m, h], sem_w.at[(j * NM + m) * 2 + h])

    def v_cp(g):
        return pltpu.make_async_copy(wqkv_hbm.at[:, pl.ds(2 * D + g * 128, 128)], wv_v.at[g], sem_v.at[g])

    wo_cp = pltpu.make_async_copy(wo_hbm, wo_v, sem_v.at[2 * NM])

    wr_cp = pltpu.make_async_copy(wr_hbm, wr_v, sem_v.at[2 * NM + 1])
    gw_cp = pltpu.make_async_copy(gw_hbm, gw_v, sem_v.at[2 * NM + 2])

    def f_cp(j, i):
        cols = pl.ds(j * FC, FC)
        if i == 2:
            return pltpu.make_async_copy(wd_hbm.at[cols], wd_v.at[cols], sem_f.at[i * NM + j])
        return pltpu.make_async_copy((wg_hbm, wu_hbm)[i].at[:, cols], (wg_v, wu_v)[i].at[j], sem_f.at[i * NM + j])

    def o_cp(t, c):
        return pltpu.make_async_copy(o_v.at[t, pl.ds(c * OC, OC)], out_hbm.at[0, pl.ds(t * TS + c * OC, OC)],
                                     sem_o.at[t * (TS // OC) + c])

    def after(words, v):
        if v is None:
            return words
        dep = zero[0] & pltpu.bitcast(v[0:8, 0:128], u32)
        r, c = words.shape
        return (words.reshape(r // 8, 8, c) | jnp.concatenate([dep] * (c // 128), axis=1)).reshape(r, c)

    def words_of(block, v):
        return after(pltpu.bitcast(block, u32), v)

    def prep_w(j, m, k, v):
        blk = [_unpack(words_of(wqk_v[j, m, h, pl.ds(i * HD + k * 128, 128), :], v)).astype(f32).T
               for h in (0, 1) for i in (0, 1)]
        for i, a in enumerate(_left(*blk)):
            (wqs_v, wks_v)[j][i, _half(m * 128, 128), pl.ds(k * 128, 128)] = _pack_mixed(a)

    def prep_x(src, dst_v, dst, r, n, v):
        blk = [words_of(x_v[src, pl.ds(h * TH + r, n), pl.ds(i * HD, HD)], v) for i in (0, 1) for h in (0, 1)]
        vals = [[pltpu.unpack_elementwise(b, index=p, packed_dtype=bf16, unpacked_dtype=f32) for b in blk]
                for p in (0, 1)]
        even, odd = _right(*vals[0]), _right(*vals[1])
        for p in (0, 1):
            for h in (0, 1):
                score = jnp.sum(vals[p][h] * top[2][:, :HD] + vals[p][2 + h] * top[2][:, HD:], axis=1, keepdims=True)
                score = score.astype(bf16).astype(f32)
                token = 2 * row8 + (src * TS + h * TH + r + p)
                better = (score > top[0]) | ((score == top[0]) & (token < top[1]))
                top[0], top[1] = jnp.where(better, score, top[0]), jnp.where(better, token, top[1])
        for i in range(7):
            dst_v[dst, i, _half(r, n), :] = blk[0] if i == 1 else blk[3] if i == 4 else _pack2(even[i], odd[i])

    def project(w_v, xs_v, u, m, work):
        rows = _half(m * MC, MC)
        return _strassen(lambda i: _dot_nt(_unpack(w_v[i, rows, :]), _unpack(xs_v[u, i])), work)

    def w_all(j, ms):
        return [w_cp(j, m, h) for m in ms for h in (0, 1)]

    def prep_ws(j, ms):
        return [lambda v, m=m, k=k: prep_w(j, m, k, v) for m in ms for k in range(HD // 128)]

    def prep_xs(t, r0, r1):
        return [lambda v, r=r: prep_x(t, (xa_v, xb_v)[t % 2], t // 2, r, 16, v) for r in range(r0, r1, 16)]

    def k_finish(t, m, c):
        c11, c12, c21, c22 = [_phi(b) for b in c]
        for h, zs in enumerate((c11 + c12, c21 + c22)):
            zr = pl.ds(h * HD + m * MC, MC)
            zs = sum(zs[:, l:l + 128] for l in range(128, TH, 128)) + zs[:, 0:128]
            zs = zs if t == 0 else z_v[zr, :] + zs
            if t == NT - 1:
                zs = jnp.broadcast_to(jnp.sum(zs, axis=1, keepdims=True), (MC, 128))
            z_v[zr, :] = zs
        for i, b in enumerate(_right(c11, c21, c12, c22)):
            ks_v[t, i, _half(m * MC, MC), :] = _pack_mixed(b)

    row8 = lax.broadcasted_iota(jnp.int32, (8, 1), 0)
    top = [jnp.full((8, 1), -jnp.inf, f32), row8, None]

    def route(_):
        best = jnp.max(top[0])
        idx = jnp.min(jnp.where(top[0] == best, top[1], S - 1))
        top[0], top[1] = best, idx
        slab = x_v[idx // TS, pl.ds(pl.multiple_of(idx % TS // 16 * 16, 16), 16), :].astype(f32)
        picked = lax.broadcasted_iota(jnp.int32, (16, D), 0) == idx % 16
        xcol_v[...] = jnp.broadcast_to(jnp.sum(jnp.where(picked, slab, 0.0), axis=0, keepdims=True), (128, D)).T

    def sync(at, waits, starts):
        def run(_):
            for cp in waits:
                cp.wait()
            for cp in starts:
                cp.start()
        return [(at, run)]

    early, end = 0.58, 0.65
    plan = {
        (0, 0): sync(0.15, w_all(1, [1]), [x_cp(1)]) + _spread(prep_ws(1, [1]), 0.15, end)
        + sync(end, w_all(1, [2]), []),
        (0, 1): _spread(prep_ws(1, [2]), 0, end) + sync(end, w_all(1, [3]), [x_cp(2)]),
        (0, 2): _spread(prep_ws(1, [3]), 0, 0.4) + sync(0.4, [x_cp(1)], [])
        + _spread(prep_xs(1, 0, 96), 0.4),
        (0, 3): _spread(prep_xs(1, 96, TH), 0, end)
        + sync(end, [x_cp(2)], [x_cp(3)] + w_all(0, range(NM))),
    }
    for m in range(NM):
        plan[1, m] = _spread(prep_xs(2, m * 64, m * 64 + 64), 0, early)
    plan[1, NM - 1] += sync(end, [x_cp(3)] + w_all(0, range(NM)),
                            [v_cp(g) for g in range(2 * NM)]
                            + [wo_cp, gw_cp, f_cp(0, 0), f_cp(0, 1)])
    for m in range(NM):
        plan[2, m] = _spread(prep_xs(3, m * 64, m * 64 + 64), 0, early)
    for m in range(NM):
        plan[3, m] = _spread(prep_ws(0, [m]), 0, early)
    plan[3, 2].append((0.5, route))

    def first_x(n):
        rows = [pl.ds(h * TH + n * TH // 2, TH // 2) for h in (0, 1)]
        return [pltpu.make_async_copy(x_hbm.at[0, rows[h]], x_v.at[0, rows[h]], sem_x.at[NT + 2 * n + h])
                for h in (0, 1)]

    for cp in [wr_cp] + first_x(0):
        cp.start()
    y_v[...] = jnp.zeros_like(y_v)
    hcol_v[pl.ds(F, FP - F), :] = jnp.zeros((FP - F, 128), f32)
    wd_v[pl.ds(F, FP - F), :] = jnp.zeros((FP - F, D), bf16)
    zero = [pltpu.bitcast(y_v[:, 0:128], u32)]
    wr_cp.wait()
    top[2] = wr_v[...].astype(f32).reshape(1, D)
    for cp in first_x(1):
        cp.start()
    for n in (0, 1):
        for cp in first_x(n):
            cp.wait()
        for cp in w_all(1, [n]):
            cp.start()
        for w in prep_xs(0, n * TH // 2, (n + 1) * TH // 2):
            w(None)
    for cp in w_all(1, [0]):
        cp.wait()
    for cp in w_all(1, [2]):
        cp.start()
    for w in prep_ws(1, [0]):
        w(None)
    for cp in w_all(1, [3]):
        cp.start()
    for (t, m), work in plan.items():
        k_finish(t, m, project(wks_v, (xa_v, xb_v)[t % 2], t // 2, m, work))

    top_r, idx = top[:2]

    def q_tile(t, u, xs_v):
        for m in range(NM):
            c = project(wqs_v, xs_v, u, m, [])
            p = []
            for i, q in enumerate(c):
                pq = _phi(q)
                zc = z_v[pl.ds((i // 2) * HD + m * MC, MC), :]
                zc = jnp.concatenate([zc] * (TH // 128), axis=1)
                den = jnp.sum((pq * zc).reshape(MC // DH, DH, TH), axis=1, keepdims=True) + 1e-6
                p.append((pq.reshape(MC // DH, DH, TH) * (1.0 / den)).reshape(MC, TH).T)
            for i, a in enumerate(_left(p[0], p[2], p[1], p[3])):
                qs_v[t, i, :, pl.ds(m * MC, MC)] = _pack(a)

    def q_body(u, carry):
        @pl.when(u == 0)
        def _():
            for j in range(1, NM):
                for i in range(2):
                    f_cp(j, i).start()

        @pl.when(u == 1)
        def _():
            for j in range(NM):
                f_cp(j, 2).start()

        q_tile(2 * u, u, xa_v)
        q_tile(2 * u + 1, u, xb_v)
        return carry

    lax.fori_loop(0, NT // 2, q_body, 0)
    for g in range(2 * NM):
        v_cp(g).wait()
    wo_cp.wait()
    gw_cp.wait()
    for j in range(NM):
        for i in range(2):
            f_cp(j, i).wait()

    def matvec(acc, w_ref, w0, col_ref, c0, n):
        for r in range(0, n, 16):
            w = w_ref[pl.ds(w0 + r, 16), :].astype(f32)
            pr = w * jnp.concatenate([col_ref[pl.ds(c0 + r, 16), :]] * (w.shape[1] // 128), axis=1)
            acc[0] = acc[0] + (pr[0:8] + pr[8:16])
        return acc[0]

    def before(words, fill):
        for w in fill:
            bits = pltpu.bitcast(w(), u32)
            dep = zero[0]
            for l in range(0, bits.shape[1], 128):
                dep = dep & bits[:, l:l + 128]
            top = words[0:8] | jnp.concatenate([dep] * (words.shape[1] // 128), axis=1)
            words = jnp.concatenate([top, words[8:]], axis=0)
        return words

    blk = (lax.broadcasted_iota(jnp.int32, (128, 128), 0) // DH) == (lax.broadcasted_iota(jnp.int32, (128, 128), 1) // DH)
    x_of = (0, 6, 1, 4, 5, 3, 2)

    def p_body(j, carry):
        ga, ua = [jnp.zeros((8, FC), f32)], [jnp.zeros((8, FC), f32)]
        fill = []
        for s in range(0, D, FR):
            fill.append(lambda s=s: matvec(ga, wg_v.at[j], s, xcol_v, s, FR))
            fill.append(lambda s=s: matvec(ua, wu_v.at[j], s, xcol_v, s, FR))
        rows = _half(j * 128, 128)

        def prod(i):
            acc = None
            for t in range(NT):
                k = i * NT + t
                lhs = before(ks_v[t, i, rows, :], fill[(k * len(fill)) // PK:((k + 1) * len(fill)) // PK])
                d = _dot(_unpack(lhs), _unpack((xa_v, xb_v)[t % 2][t // 2, x_of[i]]))
                acc = d if acc is None else acc + d
            return acc

        d11, d12, d21, d22 = _strassen(prod)
        g = jnp.sum(ga[0], axis=0, keepdims=True)
        u = jnp.sum(ua[0], axis=0, keepdims=True)
        hcol_v[pl.ds(pl.multiple_of(j * FC, 128), FC), :] = jnp.broadcast_to(g * _sigmoid(g) * u, (128, FC)).T
        for h, (lo, hi) in enumerate(((d11, d21), (d12, d22))):
            p_v[h, rows, :] = _pack_mixed(jnp.concatenate([lo, hi], axis=1))
        return carry

    lax.fori_loop(0, NM, p_body, 0)

    for j in range(NM):
        ms = []
        for h in (0, 1):
            grp = h * NM + j
            kv = _dot(_unpack(p_v[h, _half(j * 128, 128), :]), wv_v[grp])
            kv = jnp.where(blk, kv, 0.0)
            for r in range(0, 128, 8):
                kv_v[pl.ds(grp * 128 + r // 16 * 16 + r // 8 % 2, 8, stride=2), :] = kv[r:r + 8]
            kv = kv_v[pl.ds(grp * 128, 128), :].astype(bf16)
            mh = _dot(kv, wo_v[pl.ds(grp * 128, 128), :])
            ms += [mh[:, :HD], mh[:, HD:]]
        for i, b in enumerate(_right(*ms)):
            ms_v[i, _half(j * 128, 128), :] = _pack_mixed(b)

    gw = gw_v[...].astype(f32).reshape(1, D)

    def o_body(step, carry):
        t = (idx // TS + 1 + step) % NT

        @pl.when(step == 0)
        def _():
            for j in range(NM):
                f_cp(j, 2).wait()

        y = jnp.sum(y_v[...], axis=0, keepdims=True) * _sigmoid(jnp.full((1, D), top_r, f32))
        r0 = pl.multiple_of(jnp.minimum(step, NT - 2) * FO, 16)
        ya = [y_v[...]]
        fill = [lambda s=s: matvec(ya, wd_v, r0 + s, hcol_v, r0 + s, DR) for s in range(0, FO, DR)]
        nprod = 7 * (TH // OC)
        for c in range(TH // OC):
            def prod(i):
                k = 7 * c + i
                lhs = before(qs_v[t, i, _half(c * OC, OC), :],
                             fill[(k * len(fill)) // nprod:((k + 1) * len(fill)) // nprod])
                return _dot(_unpack(lhs), _unpack(ms_v[i]))

            a = _strassen(prod)
            for h in (0, 1):
                rows = pl.ds(h * TH + c * OC, OC)
                x = x_v[t, rows, :].astype(f32)
                g = _sigmoid(jnp.sum(x * gw, axis=1, keepdims=True))
                token = lax.broadcasted_iota(jnp.int32, (OC, D), 0) + (t * TS + h * TH + c * OC)
                b = jnp.where(token == idx, x + y, x)
                ah = jnp.concatenate([a[2 * h], a[2 * h + 1]], axis=1)
                o_v[t, rows, :] = (g * ah + (1.0 - g) * b).astype(bf16)
                o_cp(t, h * (TH // OC) + c).start()
        y_v[...] = ya[0]
        return carry

    lax.fori_loop(0, NT, o_body, 0)
    for t in range(NT):
        for c in range(TS // OC):
            o_cp(t, c).wait()


@jax.jit
def pallas_gated_mix__linear_attn_block__moe_arch_mod__prompt_kernel(
        A_x, A_wqkv, A_wo, B_x, B_w_r, B_w_gate, B_w_up, B_w_down, gate_w):
    del B_x
    hbm = pl.BlockSpec(memory_space=pl.ANY)
    return pl.pallas_call(
        _kernel,
        out_shape=jax.ShapeDtypeStruct((1, S, D), bf16),
        in_specs=[hbm] * 8,
        out_specs=hbm,
        scratch_shapes=[
            pltpu.VMEM((NT, TS, D), bf16),
            pltpu.VMEM((2, NM, 2, D, 128), bf16),
            pltpu.VMEM((2 * NM, D, 128), bf16),
            pltpu.VMEM((D, D), bf16),
            pltpu.VMEM((NM, D, FC), bf16),
            pltpu.VMEM((NM, D, FC), bf16),
            pltpu.VMEM((FP, D), bf16),
            pltpu.VMEM((NT // 2, 7, TH // 2, HD), u32),
            pltpu.VMEM((NT // 2, 7, TH // 2, HD), u32),
            pltpu.VMEM((7, HD // 2, HD), u32),
            pltpu.VMEM((7, HD // 2, HD), u32),
            pltpu.VMEM((NT, 7, HD // 2, TH), u32),
            pltpu.VMEM((NT, 7, TH // 2, HD), u32),
            pltpu.VMEM((2, HD // 2, D), u32),
            pltpu.VMEM((7, HD // 2, HD), u32),
            pltpu.VMEM((D, 128), f32),
            pltpu.VMEM((D + 8, 128), f32),
            pltpu.VMEM((D, 128), f32),
            pltpu.VMEM((FP, 128), f32),
            pltpu.VMEM((8, D), f32),
            pltpu.VMEM((NT, TS, D), bf16),
            pltpu.VMEM((D,), bf16),
            pltpu.VMEM((D,), bf16),
            pltpu.SemaphoreType.DMA((NT + 4,)),
            pltpu.SemaphoreType.DMA((4 * NM,)),
            pltpu.SemaphoreType.DMA((2 * NM + 3,)),
            pltpu.SemaphoreType.DMA((3 * NM,)),
            pltpu.SemaphoreType.DMA((S // OC,)),
        ],
        compiler_params=pltpu.CompilerParams(vmem_limit_bytes=110 * 1024 * 1024),
    )(A_x, A_wqkv, A_wo, B_w_r, B_w_gate, B_w_up, B_w_down, gate_w)
```
